```python
import jax
import jax.numpy as jnp

def _softmax(x, axis=-1):
    return jax.nn.softmax(x, axis=axis)

def _gelu(x):
    return jax.nn.gelu(x, approximate=True)

def _silu(x):
    return jax.nn.silu(x)

def _sigmoid(x):
    return jax.nn.sigmoid(x)

def _layernorm(x, axis=-1, eps=1e-05):
    m = jnp.mean(x, axis=axis, keepdims=True)
    v = jnp.var(x, axis=axis, keepdims=True)
    return (x - m) / jnp.sqrt(v + eps)

def _scatter_add(tgt, idx, src, axis=0):
    return tgt.at[idx].add(src)

def _segment_sum(src, seg, n):
    return jax.ops.segment_sum(src, seg, n)

class _Rng:

    def __init__(self, key):
        self._k = key

    def _next(self):
        self._k, sub = jax.random.split(self._k)
        return sub

    def normal(self, shape):
        return jax.random.normal(self._next(), shape, dtype=jnp.bfloat16)

    def randint(self, lo, hi, shape):
        return jax.random.randint(self._next(), shape, lo, hi, dtype=jnp.int32)

    def uniform(self, shape, lo=0.0, hi=1.0):
        return jax.random.uniform(self._next(), shape, jnp.bfloat16, lo, hi)

    def permutation(self, n):
        return jax.random.permutation(self._next(), n)
kernel_name = 'gated_mix__ssm_conv_h3__memory_aug_recurrent_mem_tr__prompt'

def setup_inputs():
    _rng = _Rng(jax.random.key(int.from_bytes(__import__("os").urandom(4), "little")))
    _w = lambda a: (lambda t: t.astype(jnp.bfloat16) if jnp.issubdtype(t.dtype, jnp.floating) else t)(jnp.asarray(a))

    def _A_setup():
        B, S, D = (1, 2048, 1024)
        ks = 4
        return {'q': _w((lambda *s: _rng.normal(s) * 0.05)(B, S, D)), 'k': _w((lambda *s: _rng.normal(s) * 0.05)(B, S, D)), 'v': _w((lambda *s: _rng.normal(s) * 0.05)(B, S, D)), 'shift_k': _w((lambda *s: _rng.normal(s) * 0.05)(D, ks) * 0.5), 'ssm_k': _w((lambda *s: _rng.normal(s) * 0.05)(D, S) * (1.0 / S ** 0.5)), 'ssm_D': _w((lambda *s: _rng.normal(s) * 0.05)(D))}
    _A_in = _A_setup()

    def _B_setup():
        B, S, Dm = (1, 2048, 1024)
        H, Dh = (32, 128)
        M, seg = (8, 32)
        seg = min(seg, S)
        S = S // seg * seg
        return {'x': _w((lambda *s: _rng.normal(s) * 0.05)(B, S, Dm)), 'mem0': _w((lambda *s: _rng.normal(s) * 0.05)(B, M, Dm)), 'Wq': _w((lambda *s: _rng.normal(s) * 0.05)(Dm, H, Dh) * Dm ** (-0.5)), 'Wk': _w((lambda *s: _rng.normal(s) * 0.05)(Dm, H, Dh) * Dm ** (-0.5)), 'Wv': _w((lambda *s: _rng.normal(s) * 0.05)(Dm, H, Dh) * Dm ** (-0.5)), 'Wo': _w((lambda *s: _rng.normal(s) * 0.05)(H, Dh, Dm) * (H * Dh) ** (-0.5)), 'seg_len': seg}
    _B_in = _B_setup()
    return {'A_q': _A_in['q'], 'A_k': _A_in['k'], 'A_v': _A_in['v'], 'A_shift_k': _A_in['shift_k'], 'A_ssm_k': _A_in['ssm_k'], 'A_ssm_D': _A_in['ssm_D'], 'B_x': _B_in['x'], 'B_mem0': _B_in['mem0'], 'B_Wq': _B_in['Wq'], 'B_Wk': _B_in['Wk'], 'B_Wv': _B_in['Wv'], 'B_Wo': _B_in['Wo'], 'B_seg_len': _B_in['seg_len'], 'gate_w': _w((lambda *s: _rng.normal(s) * 0.05)(1024))}

def reference(A_q, A_k, A_v, A_shift_k, A_ssm_k, A_ssm_D, B_x, B_mem0, B_Wq, B_Wk, B_Wv, B_Wo, B_seg_len, gate_w):

    def _A_ref(q, k, v, shift_k, ssm_k, ssm_D):
        B, S, D = q.shape
        ks = shift_k.shape[-1]
        k_pad = jnp.pad(k, ((0, 0), (ks - 1, 0), (0, 0)))
        k_shift = jnp.zeros_like(k)
        for t in range(ks):
            k_shift = k_shift + k_pad[:, t:t + S, :] * shift_k[:, ks - 1 - t][None, None, :]
        kv = k_shift * v
        L = 2 * S
        kv_pad = jnp.pad(kv, ((0, 0), (0, S), (0, 0)))
        kf_pad = jnp.pad(ssm_k, ((0, 0), (0, S)))
        kv_f = (lambda x, axes=(-2, -1): jnp.fft.rfft2(x.astype(jnp.float32), axes=axes))(kv_pad[:, None, :, :], axes=(1, 2))
        kf_f = (lambda x, axes=(-2, -1): jnp.fft.rfft2(x.astype(jnp.float32), axes=axes))(kf_pad[:, None, :], axes=(1, 2))
        kf_f = (lambda x, *d: x.transpose(*d))(kf_f, 1, 2, 0)
        y_f = kv_f * kf_f[None, :, :, :]
        y = (lambda x, s, axes=(-2, -1): jnp.fft.irfft2(x, s=s, axes=axes).astype(jnp.bfloat16))(y_f, (1, L), axes=(1, 2))[:, 0, :S, :]
        y = y + kv * ssm_D[None, None, :]
        return q * y

    def _B_ref(x, mem0, Wq, Wk, Wv, Wo, seg_len):
        B, S, Dm = x.shape
        H, Dh = (Wq.shape[1], Wq.shape[2])
        M = mem0.shape[1]
        scale = Dh ** (-0.5)
        n_seg = S // seg_len
        L = M + seg_len
        idx = jnp.arange(L)
        mask = (idx[:, None] < M) | (idx[:, None] >= idx[None, :])
        mem = mem0
        outs = []
        for s in range(n_seg):
            xs = x[:, s * seg_len:(s + 1) * seg_len, :].copy()
            h = jnp.concatenate([mem, xs], axis=1)
            q = jnp.einsum('btd,dhe->bhte', h, Wq)
            k = jnp.einsum('btd,dhe->bhte', h, Wk)
            v = jnp.einsum('btd,dhe->bhte', h, Wv)
            scores = jnp.einsum('bhqe,bhke->bhqk', q, k) * scale
            scores = jnp.where(mask[None, None], scores, -1000000000.0)
            p = _softmax(scores, axis=-1)
            o = jnp.einsum('bhqk,bhke->bhqe', p, v)
            o = jnp.einsum('bhte,hed->btd', o, Wo)
            mem = o[:, :M, :].copy()
            outs.append(o[:, M:, :])
        return jnp.concatenate(outs, axis=1)
    x = A_q
    g = _sigmoid((x * gate_w).sum(-1, keepdims=True))
    a = _A_ref(x, A_k, A_v, A_shift_k, A_ssm_k, A_ssm_D)
    b = _B_ref(x, B_mem0, B_Wq, B_Wk, B_Wv, B_Wo, B_seg_len)
    return g * a + (1 - g) * b
```

```python
import functools

import numpy as np
import jax
import jax.numpy as jnp
import jax.experimental.pallas as pl
import jax.experimental.pallas.tpu as pltpu

F32 = jnp.float32
BF16 = jnp.bfloat16
U32 = jnp.uint32

S = 2048
D = 1024
NH = 32
DH = 128
MEM = 8
SEG = 32
NSEG = S // SEG
L = MEM + SEG

TB = 256
NB = S // TB
CC = 256
DCH = 128
HG = 8


def _dft_consts():
    n = 2 * TB
    t = np.arange(TB, dtype=np.float64)[None, :]
    f = (np.arange(TB, dtype=np.float64) + 0.5)[:, None]
    ang = 2.0 * np.pi * t * f / n
    fwd = np.concatenate([np.cos(ang), -np.sin(ang)], axis=0)
    inv = np.concatenate([np.cos(ang).T, -np.sin(ang).T], axis=1) * (2.0 / n)
    sgn = np.where(np.arange(TB) % 2 == 0, 1.0, -1.0)[:, None] * np.ones((1, 128))
    return fwd.astype(np.float32), inv.astype(np.float32), sgn.astype(np.float32)


def _nt(a, b):
    return jax.lax.dot_general(a, b, (((1,), (1,)), ((), ())), preferred_element_type=F32)


def _nn(a, b):
    return jax.lax.dot_general(a, b, (((1,), (0,)), ((), ())), preferred_element_type=F32)


def _kernel(xq_hbm, k_hbm, v_hbm, ssmk_hbm, wq_hbm, wk_hbm, wv_hbm, wo_hbm,
            shift_ref, ssmd_ref, gate_ref, mem0_ref, fwd_ref, inv_ref, sgn_ref,
            o_hbm,
            x_ref, y_ref, w2_ref, wo2_ref, out_ref, sem_in, sem_w, sem_out):
    def phase_a(k_ref, v_ref, ssmk_ref, kpad_ref, kv_ref, uh_ref, kh_ref, stage_ref, stage_o_ref):
        in_copies = [
            pltpu.make_async_copy(k_hbm, k_ref, sem_in.at[0]),
            pltpu.make_async_copy(v_hbm, v_ref, sem_in.at[1]),
            pltpu.make_async_copy(ssmk_hbm, ssmk_ref, sem_in.at[2]),
            pltpu.make_async_copy(xq_hbm, x_ref, sem_in.at[3]),
        ]
        for c in in_copies:
            c.start()

        n_dch = D // DCH
        w_hbms = (wq_hbm, wk_hbm, wv_hbm)
        jobs = [(m, c) for m in range(3) for c in range(n_dch)]
        nbuf = stage_ref.shape[0]

        def w_copy(i):
            m, c = jobs[i]
            return pltpu.make_async_copy(
                w_hbms[m].at[pl.ds(c * DCH * NH, DCH * NH), :], stage_ref.at[i % nbuf], sem_w.at[i % nbuf])

        wo_copy = pltpu.make_async_copy(wo_hbm, stage_o_ref, sem_w.at[nbuf])
        for i in range(nbuf):
            w_copy(i).start()

        def retile(i):
            m, c = jobs[i]
            w_copy(i).wait()
            u_ref = stage_ref.at[i % nbuf].bitcast(U32)
            for j in range(NH // 2):
                for b in range(DCH // 16):
                    r0 = b * 16 * (NH // 2) + j
                    ev = u_ref[pl.ds(r0, 8, stride=NH), :]
                    od = u_ref[pl.ds(r0 + NH // 2, 8, stride=NH), :]
                    lo = (ev & jnp.uint32(0xFFFF)) | (od << 16)
                    hi = (ev >> 16) | (od & jnp.uint32(0xFFFF0000))
                    row = c * (DCH // 2) + 8 * b
                    w2_ref[pl.ds(row, 8), pl.ds(((2 * j) * 3 + m) * DH, DH)] = lo
                    w2_ref[pl.ds(row, 8), pl.ds(((2 * j + 1) * 3 + m) * DH, DH)] = hi
            if i + nbuf < len(jobs):
                w_copy(i + nbuf).start()
            elif i + nbuf == len(jobs):
                wo_copy.start()

        in_copies[0].wait()
        in_copies[1].wait()
        in_copies[2].wait()

        kpad_ref[pl.ds(0, 8), :] = jnp.zeros((8, CC), F32)
        sgn = sgn_ref[...]
        sgn = jnp.concatenate([sgn] * (CC // 128), axis=1)
        n_cc = D // CC
        per = len(jobs) // n_cc
        for cc in range(n_cc):
            cs = pl.ds(cc * CC, CC)
            kpad_ref[pl.ds(8, S), :] = k_ref[:, cs].astype(F32)
            for j in range(NB):
                acc = None
                for tap in range(4):
                    w = shift_ref[pl.ds(tap, 1), cs].astype(F32)
                    term = kpad_ref[pl.ds(8 + j * TB - tap, TB), :] * w
                    acc = term if acc is None else acc + term
                kvb = (acc * v_ref[pl.ds(j * TB, TB), cs].astype(F32)).astype(BF16)
                kv_ref[pl.ds(j * TB, TB), :] = kvb
                uh_ref[j] = _nn(fwd_ref[...], kvb)
                kh_ref[j] = _nt(fwd_ref[...], ssmk_ref[cs, pl.ds(j * TB, TB)])
            for m in range(NB - 1, 0, -1):
                pr = kh_ref[m - 1, pl.ds(0, TB), :]
                pi = kh_ref[m - 1, pl.ds(TB, TB), :]
                kh_ref[m, pl.ds(0, TB), :] = kh_ref[m, pl.ds(0, TB), :] - sgn * pi
                kh_ref[m, pl.ds(TB, TB), :] = kh_ref[m, pl.ds(TB, TB), :] + sgn * pr
            dcoef = ssmd_ref[:, cs].astype(F32)
            for i in range(NB):
                zr = None
                zi = None
                for m in range(i + 1):
                    kr = kh_ref[m, pl.ds(0, TB), :]
                    ki = kh_ref[m, pl.ds(TB, TB), :]
                    ur = uh_ref[i - m, pl.ds(0, TB), :]
                    ui = uh_ref[i - m, pl.ds(TB, TB), :]
                    tr = kr * ur - ki * ui
                    ti = kr * ui + ki * ur
                    zr = tr if zr is None else zr + tr
                    zi = ti if zi is None else zi + ti
                z = jnp.concatenate([zr, zi], axis=0).astype(BF16)
                yb = _nn(inv_ref[...], z)
                yb = yb + kv_ref[pl.ds(i * TB, TB), :].astype(F32) * dcoef
                y_ref[pl.ds(i * TB, TB), cs] = yb.astype(BF16)
            for i in range(cc * per, (cc + 1) * per):
                retile(i)

        wo_copy.wait()
        for b in range(D * 4 // 256):
            wo2_ref[pl.ds(b * 128, 128), :] = pltpu.bitcast(stage_o_ref[pl.ds(b * 256, 256), :], U32)
        in_copies[3].wait()

    pl.run_scoped(
        phase_a,
        pltpu.VMEM((S, D), BF16), pltpu.VMEM((S, D), BF16), pltpu.VMEM((D, S), BF16),
        pltpu.VMEM((S + 8, CC), F32), pltpu.VMEM((S, CC), BF16),
        pltpu.VMEM((NB, 2 * TB, CC), F32), pltpu.VMEM((NB, 2 * TB, CC), F32),
        pltpu.VMEM((4, DCH * NH, DH), BF16), pltpu.VMEM((NH * DH, D), BF16),
    )

    scale = DH ** -0.5
    row = jax.lax.broadcasted_iota(jnp.int32, (L, L), 0)
    col = jax.lax.broadcasted_iota(jnp.int32, (L, L), 1)
    mask = (row < MEM) | (row >= col)

    def out_copy(s):
        r = pl.multiple_of(s * SEG, SEG)
        return pltpu.make_async_copy(out_ref.at[pl.ds(r, SEG), :], o_hbm.at[pl.ds(r, SEG), :], sem_out)

    def seg_body(s, mem):
        r = pl.multiple_of(s * SEG, SEG)
        xs = x_ref[pl.ds(r, SEG), :].astype(F32)
        h = jnp.concatenate([mem, xs], axis=0)
        acc = None
        for g in range(NH // HG):
            wg = pltpu.bitcast(w2_ref[:, pl.ds(g * HG * 3 * DH, HG * 3 * DH)], BF16)
            qkv = _nn(h, wg)
            os_ = []
            for hh in range(HG):
                q = qkv[:, (3 * hh) * DH:(3 * hh + 1) * DH].astype(BF16)
                k = qkv[:, (3 * hh + 1) * DH:(3 * hh + 2) * DH].astype(BF16)
                v = qkv[:, (3 * hh + 2) * DH:(3 * hh + 3) * DH].astype(BF16)
                sc = _nt(q, k) * scale
                sc = jnp.where(mask, sc, -1e9)
                mx = jnp.max(sc, axis=-1, keepdims=True)
                e = jnp.exp(sc - mx)
                p = e / jnp.sum(e, axis=-1, keepdims=True)
                o = _nn(p.astype(BF16), v)
                os_.append(o.astype(BF16).astype(F32))
            og = jnp.concatenate(os_, axis=1)
            wog = pltpu.bitcast(wo2_ref[pl.ds(g * HG * DH // 2, HG * DH // 2), :], BF16)
            part = _nn(og, wog)
            acc = part if acc is None else acc + part
        ob = acc.astype(BF16)
        mem_next = ob[:MEM].astype(F32)
        b = ob[MEM:].astype(F32)
        gsum = jnp.sum((xs * gate_ref[...].astype(F32)).astype(BF16).astype(F32), axis=-1, keepdims=True)
        gte = jax.nn.sigmoid(gsum.astype(BF16).astype(F32))
        a = (xs * y_ref[pl.ds(r, SEG), :].astype(F32)).astype(BF16).astype(F32)
        out_ref[pl.ds(r, SEG), :] = (gte * a + (1.0 - gte) * b).astype(BF16)
        out_copy(s).start()
        return mem_next

    jax.lax.fori_loop(0, NSEG, seg_body, mem0_ref[...].astype(F32))
    pltpu.make_async_copy(out_ref, o_hbm, sem_out).wait()


@functools.partial(jax.jit, static_argnames=("B_seg_len",))
def pallas_gated_mix__ssm_conv_h3__memory_aug_recurrent_mem_tr__prompt_kernel(
    A_q, A_k, A_v, A_shift_k, A_ssm_k, A_ssm_D, B_x, B_mem0, B_Wq, B_Wk, B_Wv, B_Wo, B_seg_len, gate_w,
):
    del B_x
    assert B_seg_len == SEG
    fwd, inv, sgn = _dft_consts()
    any_spec = pl.BlockSpec(memory_space=pl.ANY)
    vmem_spec = pl.BlockSpec(memory_space=pltpu.VMEM)
    out = pl.pallas_call(
        _kernel,
        out_shape=jax.ShapeDtypeStruct((S, D), BF16),
        in_specs=[any_spec] * 8 + [vmem_spec] * 7,
        out_specs=any_spec,
        scratch_shapes=[
            pltpu.VMEM((S, D), BF16),
            pltpu.VMEM((S, D), BF16),
            pltpu.VMEM((D // 2, 3 * NH * DH), U32),
            pltpu.VMEM((NH * DH // 2, D), U32),
            pltpu.VMEM((S, D), BF16),
            pltpu.SemaphoreType.DMA((4,)),
            pltpu.SemaphoreType.DMA((5,)),
            pltpu.SemaphoreType.DMA(()),
        ],
        compiler_params=pltpu.CompilerParams(vmem_limit_bytes=120 * 1024 * 1024),
    )(
        A_q.reshape(S, D), A_k.reshape(S, D), A_v.reshape(S, D), A_ssm_k,
        B_Wq.reshape(D * NH, DH), B_Wk.reshape(D * NH, DH), B_Wv.reshape(D * NH, DH),
        B_Wo.reshape(NH * DH, D),
        A_shift_k.T, A_ssm_D.reshape(1, D), gate_w.reshape(1, D), B_mem0.reshape(MEM, D),
        jnp.asarray(fwd.astype(jnp.bfloat16)), jnp.asarray(inv.astype(jnp.bfloat16)), jnp.asarray(sgn),
    )
    return out.reshape(1, S, D)
```

```python
import functools

import numpy as np
import jax
import jax.numpy as jnp
import jax.experimental.pallas as pl
import jax.experimental.pallas.tpu as pltpu

F32 = jnp.float32
BF16 = jnp.bfloat16
U32 = jnp.uint32

S = 2048
D = 1024
NH = 32
DH = 128
MEM = 8
SEG = 32
NSEG = S // SEG
L = MEM + SEG

TB = 256
NB = S // TB
CC = 256
DCH = 128
HG = 2
LAG = 2
TAIL = 2
TAILPOS = 4
WOG = 4


def _dft_consts():
    n = 2 * TB
    t = np.arange(TB, dtype=np.float64)[None, :]
    f = (np.arange(TB, dtype=np.float64) + 0.5)[:, None]
    ang = 2.0 * np.pi * t * f / n
    fwd = np.concatenate([np.cos(ang), -np.sin(ang)], axis=0)
    inv = np.concatenate([np.cos(ang).T, -np.sin(ang).T], axis=1) * (2.0 / n)
    sgn = np.where(np.arange(TB) % 2 == 0, 1.0, -1.0)[:, None] * np.ones((1, 128))
    return fwd.astype(np.float32), inv.astype(np.float32), sgn.astype(np.float32)


def _nt(a, b):
    return jax.lax.dot_general(a, b, (((1,), (1,)), ((), ())), preferred_element_type=F32)


def _nn(a, b):
    return jax.lax.dot_general(a, b, (((1,), (0,)), ((), ())), preferred_element_type=F32)


def _kernel(xq_hbm, k_hbm, v_hbm, ssmk_hbm, wq_hbm, wk_hbm, wv_hbm, wo_hbm,
            shift_ref, ssmd_ref, gate_ref, mem0_ref, fwd_ref, inv_ref, sgn_ref,
            o_hbm,
            x_ref, y_ref, w2_ref, wo2_ref, out_ref, sem_in, sem_w, sem_out):
    def phase_a(k_ref, v_ref, ssmk_ref, kpad_ref, kv_ref, uh_ref, kh_ref, stage_ref, stage_o_ref):
        n_cc = D // CC
        w_hbms = (wq_hbm, wk_hbm, wv_hbm)
        cpg = D // DCH // n_cc

        def in_copies(cc):
            c0 = pl.multiple_of(cc * CC, CC)
            return (
                pltpu.make_async_copy(k_hbm.at[:, pl.ds(c0, CC)], k_ref.at[:, pl.ds(c0, CC)], sem_in.at[3 * cc]),
                pltpu.make_async_copy(v_hbm.at[:, pl.ds(c0, CC)], v_ref.at[:, pl.ds(c0, CC)], sem_in.at[3 * cc + 1]),
                pltpu.make_async_copy(ssmk_hbm.at[pl.ds(c0, CC), :], ssmk_ref.at[pl.ds(c0, CC), :],
                                      sem_in.at[3 * cc + 2]),
            )

        def w_copy(cc, m, i):
            r0 = pl.multiple_of((cc * cpg + i) * (DCH * NH), DCH * NH)
            return pltpu.make_async_copy(
                w_hbms[m].at[pl.ds(r0, DCH * NH), :], stage_ref.at[m * cpg + i], sem_w.at[m * cpg + i])

        x_copy = pltpu.make_async_copy(xq_hbm, x_ref, sem_in.at[3 * n_cc])
        wo_copy = pltpu.make_async_copy(wo_hbm, stage_o_ref, sem_w.at[3 * cpg])

        def retile(jj, cc):
            m = jj // cpg
            c = cc * cpg + jj % cpg
            u_ref = stage_ref.at[jj].bitcast(U32)
            for j in range(NH // 2):
                c0 = pl.multiple_of((2 * j * 3 + m) * DH, DH)
                c1 = pl.multiple_of(((2 * j + 1) * 3 + m) * DH, DH)
                for b in range(DCH // 16):
                    r0 = b * 16 * (NH // 2) + j
                    ev = u_ref[pl.ds(r0, 8, stride=NH), :]
                    od = u_ref[pl.ds(r0 + NH // 2, 8, stride=NH), :]
                    lo = (ev & jnp.uint32(0xFFFF)) | (od << 16)
                    hi = (ev >> 16) | (od & jnp.uint32(0xFFFF0000))
                    row = pl.multiple_of(c * (DCH // 2) + 8 * b, 8)
                    w2_ref[pl.ds(row, 8), pl.ds(c0, DH)] = lo
                    w2_ref[pl.ds(row, 8), pl.ds(c1, DH)] = hi

        for c in in_copies(0):
            c.start()
        kpad_ref[pl.ds(0, 8), :] = jnp.zeros((8, CC), F32)

        def chunk(cc, _):
            @pl.when(cc + 1 < n_cc)
            def _():
                for c in in_copies(cc + 1):
                    c.start()
            for m in range(3):
                for i in range(cpg):
                    w_copy(cc, m, i).start()

            @pl.when(cc == 1)
            def _():
                wo_copy.start()

            @pl.when(cc == 2)
            def _():
                x_copy.start()

            for c in in_copies(cc):
                c.wait()
            cs = pl.ds(pl.multiple_of(cc * CC, CC), CC)
            kpad_ref[pl.ds(8, S), :] = k_ref[:, cs].astype(F32)

            def fwd_block(j, _):
                t0 = pl.multiple_of(j * TB, TB)
                acc = None
                win = kpad_ref[pl.ds(t0, TB + 8), :]
                for tap in range(4):
                    w = shift_ref[pl.ds(tap, 1), cs].astype(F32)
                    term = win[8 - tap:8 - tap + TB, :] * w
                    acc = term if acc is None else acc + term
                kvb = (acc * v_ref[pl.ds(t0, TB), cs].astype(F32)).astype(BF16)
                kv_ref[pl.ds(t0, TB), :] = kvb
                uh_ref[j] = _nn(fwd_ref[...], kvb)
                kh_ref[j] = _nt(fwd_ref[...], ssmk_ref[cs, pl.ds(t0, TB)])
                return 0

            jax.lax.fori_loop(0, NB, fwd_block, 0)

            sgn = sgn_ref[pl.ds(0, 8), :]

            def spec_tile(ft, _):
                f0 = pl.multiple_of(ft * 8, 8)
                for lc in range(CC // 128):
                    ls = pl.ds(lc * 128, 128)
                    kr0 = [kh_ref[m, pl.ds(f0, 8), ls] for m in range(NB)]
                    ki0 = [kh_ref[m, pl.ds(TB + f0, 8), ls] for m in range(NB)]
                    kr = [kr0[0]] + [kr0[m] - sgn * ki0[m - 1] for m in range(1, NB)]
                    ki = [ki0[0]] + [ki0[m] + sgn * kr0[m - 1] for m in range(1, NB)]
                    ur = [uh_ref[j, pl.ds(f0, 8), ls] for j in range(NB)]
                    ui = [uh_ref[j, pl.ds(TB + f0, 8), ls] for j in range(NB)]
                    for i in range(NB):
                        zr = None
                        zi = None
                        for m in range(i + 1):
                            tr = kr[m] * ur[i - m] - ki[m] * ui[i - m]
                            ti = kr[m] * ui[i - m] + ki[m] * ur[i - m]
                            zr = tr if zr is None else zr + tr
                            zi = ti if zi is None else zi + ti
                        kh_ref[i, pl.ds(f0, 8), ls] = zr
                        kh_ref[i, pl.ds(TB + f0, 8), ls] = zi
                return 0

            jax.lax.fori_loop(0, TB // 8, spec_tile, 0)

            def inv_block(i, _):
                t0 = pl.multiple_of(i * TB, TB)
                yb = _nn(inv_ref[...], kh_ref[i].astype(BF16))
                yb = yb + kv_ref[pl.ds(t0, TB), :].astype(F32) * ssmd_ref[:, cs].astype(F32)
                y_ref[pl.ds(t0, TB), cs] = yb.astype(BF16)
                return 0

            jax.lax.fori_loop(0, NB, inv_block, 0)

            for m in range(3):
                for i in range(cpg):
                    w_copy(cc, m, i).wait()
            jax.lax.fori_loop(0, 3 * cpg, lambda jj, c: (retile(jj, cc), c)[1], 0)
            return 0

        jax.lax.fori_loop(0, n_cc, chunk, 0)

        wo_copy.wait()

        def wo_retile(b, _):
            wo2_ref[pl.ds(pl.multiple_of(b * 128, 128), 128), :] = pltpu.bitcast(
                stage_o_ref[pl.ds(pl.multiple_of(b * 256, 256), 256), :], U32)
            return 0

        jax.lax.fori_loop(0, D * 4 // 256, wo_retile, 0)
        x_copy.wait()

    pl.run_scoped(
        phase_a,
        pltpu.VMEM((S, D), BF16), pltpu.VMEM((S, D), BF16), pltpu.VMEM((D, S), BF16),
        pltpu.VMEM((S + 8, CC), F32), pltpu.VMEM((S, CC), BF16),
        pltpu.VMEM((NB, 2 * TB, CC), F32), pltpu.VMEM((NB, 2 * TB, CC), F32),
        pltpu.VMEM((3 * (CC // DCH), DCH * NH, DH), BF16), pltpu.VMEM((NH * DH, D), BF16),
    )

    scale = DH ** -0.5
    row = jax.lax.broadcasted_iota(jnp.int32, (L, L), 0)
    col = jax.lax.broadcasted_iota(jnp.int32, (L, L), 1)
    mask = (row < MEM) | (row >= col)

    def out_copy(s):
        r = pl.multiple_of(s * SEG, SEG)
        return pltpu.make_async_copy(out_ref.at[pl.ds(r, SEG), :], o_hbm.at[pl.ds(r, SEG), :], sem_out)

    def seg_body(s, mem):
        r = pl.multiple_of(s * SEG, SEG)
        xs = x_ref[pl.ds(r, SEG), :].astype(F32)
        h = jnp.concatenate([mem, xs], axis=0)
        ngrp = NH // HG
        qkvs = [None] * ngrp
        os_ = [None] * NH

        def attend(g):
            qkv = qkvs[g]
            for hh in range(HG):
                q = qkv[:, (3 * hh) * DH:(3 * hh + 1) * DH].astype(BF16).astype(F32)
                k = qkv[:, (3 * hh + 1) * DH:(3 * hh + 2) * DH].astype(BF16)
                v = qkv[:, (3 * hh + 2) * DH:(3 * hh + 3) * DH].astype(BF16)
                sc = _nt(q, k) * scale
                sc = jnp.where(mask, sc, -1e9)
                mx = jnp.max(sc, axis=-1, keepdims=True)
                e = jnp.exp(sc - mx)
                p = e / jnp.sum(e, axis=-1, keepdims=True)
                o = _nn(p.astype(BF16).astype(F32), v)
                os_[g * HG + hh] = o.astype(BF16).astype(F32)

        for g in range(ngrp + LAG):
            if g < ngrp:
                wg = pltpu.bitcast(w2_ref[:, pl.ds(g * HG * 3 * DH, HG * 3 * DH)], BF16)
                qkvs[g] = _nn(h, wg)
            if g >= LAG and g - LAG < ngrp - TAIL:
                attend(g - LAG)
        acc = None
        nwo = NH // WOG
        for g in range(nwo):
            if g == nwo - 1 - TAILPOS:
                for t in range(ngrp - TAIL, ngrp):
                    attend(t)
            og = jnp.concatenate(os_[g * WOG:(g + 1) * WOG], axis=1)
            wog = pltpu.bitcast(wo2_ref[pl.ds(g * WOG * DH // 2, WOG * DH // 2), :], BF16)
            part = _nn(og, wog)
            acc = part if acc is None else acc + part
        ob = acc.astype(BF16)
        mem_next = ob[:MEM].astype(F32)
        b = ob[MEM:].astype(F32)
        gsum = jnp.sum((xs * gate_ref[...].astype(F32)).astype(BF16).astype(F32), axis=-1, keepdims=True)
        gte = jax.nn.sigmoid(gsum.astype(BF16).astype(F32))
        a = (xs * y_ref[pl.ds(r, SEG), :].astype(F32)).astype(BF16).astype(F32)
        out_ref[pl.ds(r, SEG), :] = (gte * a + (1.0 - gte) * b).astype(BF16)
        out_copy(s).start()
        return mem_next

    jax.lax.fori_loop(0, NSEG, seg_body, mem0_ref[...].astype(F32))
    pltpu.make_async_copy(out_ref, o_hbm, sem_out).wait()


@functools.partial(jax.jit, static_argnames=("B_seg_len",))
def pallas_gated_mix__ssm_conv_h3__memory_aug_recurrent_mem_tr__prompt_kernel(
    A_q, A_k, A_v, A_shift_k, A_ssm_k, A_ssm_D, B_x, B_mem0, B_Wq, B_Wk, B_Wv, B_Wo, B_seg_len, gate_w,
):
    del B_x
    assert B_seg_len == SEG
    fwd, inv, sgn = _dft_consts()
    any_spec = pl.BlockSpec(memory_space=pl.ANY)
    vmem_spec = pl.BlockSpec(memory_space=pltpu.VMEM)
    out = pl.pallas_call(
        _kernel,
        out_shape=jax.ShapeDtypeStruct((S, D), BF16),
        in_specs=[any_spec] * 8 + [vmem_spec] * 7,
        out_specs=any_spec,
        scratch_shapes=[
            pltpu.VMEM((S, D), BF16),
            pltpu.VMEM((S, D), BF16),
            pltpu.VMEM((D // 2, 3 * NH * DH), U32),
            pltpu.VMEM((NH * DH // 2, D), U32),
            pltpu.VMEM((S, D), BF16),
            pltpu.SemaphoreType.DMA((3 * (D // CC) + 1,)),
            pltpu.SemaphoreType.DMA((3 * (CC // DCH) + 1,)),
            pltpu.SemaphoreType.DMA(()),
        ],
        compiler_params=pltpu.CompilerParams(vmem_limit_bytes=120 * 1024 * 1024),
    )(
        A_q.reshape(S, D), A_k.reshape(S, D), A_v.reshape(S, D), A_ssm_k,
        B_Wq.reshape(D * NH, DH), B_Wk.reshape(D * NH, DH), B_Wv.reshape(D * NH, DH),
        B_Wo.reshape(NH * DH, D),
        A_shift_k.T, A_ssm_D.reshape(1, D), gate_w.reshape(1, D), B_mem0.reshape(MEM, D),
        jnp.asarray(fwd.astype(jnp.bfloat16)), jnp.asarray(inv.astype(jnp.bfloat16)), jnp.asarray(sgn),
    )
    return out.reshape(1, S, D)
```

```python
import functools

import numpy as np
import jax
import jax.numpy as jnp
import jax.experimental.pallas as pl
import jax.experimental.pallas.tpu as pltpu

F32 = jnp.float32
BF16 = jnp.bfloat16
U32 = jnp.uint32

S = 2048
D = 1024
NH = 32
DH = 128
MEM = 8
SEG = 32
NSEG = S // SEG
L = MEM + SEG

TB = 256
NB = S // TB
CC = 256
DCH = 128
WPITCH = 24
WO_AT = 1
XSPLIT = 128
UNR = 4
HG = 2
LAG = 2
TAIL = 2
TAILPOS = 4
WOG = 4
EPI = 1


def _dft_consts():
    n = 2 * TB
    t = np.arange(TB, dtype=np.float64)[None, :]
    f = (np.arange(TB, dtype=np.float64) + 0.5)[:, None]
    ang = 2.0 * np.pi * t * f / n
    fwd = np.concatenate([np.cos(ang), -np.sin(ang)], axis=0)
    inv = np.concatenate([np.cos(ang).T, -np.sin(ang).T], axis=1) * (2.0 / n)
    sgn = np.where(np.arange(TB) % 2 == 0, 1.0, -1.0)[:, None] * np.ones((1, 128))
    return fwd.astype(np.float32), inv.astype(np.float32), sgn.astype(np.float32)


def _nt(a, b):
    return jax.lax.dot_general(a, b, (((1,), (1,)), ((), ())), preferred_element_type=F32)


def _nn(a, b):
    return jax.lax.dot_general(a, b, (((1,), (0,)), ((), ())), preferred_element_type=F32)


def unrolled(body):
    def run(j, c):
        for u in range(UNR):
            body(UNR * j + u, c)
        return c
    return run


def _kernel(xq_hbm, k_hbm, v_hbm, ssmk_hbm, wq_hbm, wk_hbm, wv_hbm, wo_hbm,
            shift_ref, ssmd_ref, gate_ref, mem0_ref, fwd_ref, inv_ref, sgn_ref,
            o_hbm,
            x_ref, y_ref, w2_ref, wo2_ref, out_ref, b_ref, sem_in, sem_w, sem_x, sem_out):
    x_copies = [
        pltpu.make_async_copy(xq_hbm.at[pl.ds(0, XSPLIT), :], x_ref.at[pl.ds(0, XSPLIT), :], sem_x.at[0]),
        pltpu.make_async_copy(xq_hbm.at[pl.ds(XSPLIT, S - XSPLIT), :], x_ref.at[pl.ds(XSPLIT, S - XSPLIT), :],
                              sem_x.at[1]),
    ]

    def phase_a(k_ref, v_ref, ssmk_ref, kpad_ref, kv_ref, uh_ref, kh_ref, stage_ref, stage_o_ref):
        n_cc = D // CC
        w_hbms = (wq_hbm, wk_hbm, wv_hbm)
        cpg = D // DCH // n_cc

        def in_copies(cc):
            c0 = pl.multiple_of(cc * CC, CC)
            return (
                pltpu.make_async_copy(k_hbm.at[:, pl.ds(c0, CC)], k_ref.at[:, pl.ds(c0, CC)], sem_in.at[3 * cc]),
                pltpu.make_async_copy(v_hbm.at[:, pl.ds(c0, CC)], v_ref.at[:, pl.ds(c0, CC)], sem_in.at[3 * cc + 1]),
                pltpu.make_async_copy(ssmk_hbm.at[pl.ds(c0, CC), :], ssmk_ref.at[pl.ds(c0, CC), :],
                                      sem_in.at[3 * cc + 2]),
            )

        def w_copies(cc, m, i):
            src = w_hbms[m].bitcast(U32)
            r0 = pl.multiple_of((cc * cpg + i) * (DCH // 2), DCH // 2)
            job = m * cpg + i
            return [
                pltpu.make_async_copy(
                    src.at[pl.ds(r0, DCH // 2), pl.ds(par * (NH // 2), NH // 2), :],
                    stage_ref.at[2 * job + par, :, pl.ds(0, NH // 2), :], sem_w.at[2 * job + par])
                for par in range(2)
            ]

        wo_copy = pltpu.make_async_copy(wo_hbm, stage_o_ref, sem_w.at[6 * cpg])

        def retile(m, i, cc):
            jj = m * cpg + i
            c = cc * cpg + i
            ev_ref = stage_ref.at[2 * jj].reshape(DCH // 2 * WPITCH, DH)
            od_ref = stage_ref.at[2 * jj + 1].reshape(DCH // 2 * WPITCH, DH)
            for j in range(NH // 2):
                c0 = pl.multiple_of((2 * j * 3 + m) * DH, DH)
                c1 = pl.multiple_of(((2 * j + 1) * 3 + m) * DH, DH)
                for b in range(DCH // 16):
                    r0 = b * 8 * WPITCH + j
                    ev = ev_ref[pl.ds(r0, 8, stride=WPITCH), :]
                    od = od_ref[pl.ds(r0, 8, stride=WPITCH), :]
                    lo = (ev & jnp.uint32(0xFFFF)) | (od << 16)
                    hi = (ev >> 16) | (od & jnp.uint32(0xFFFF0000))
                    row = pl.multiple_of(c * (DCH // 2) + 8 * b, 8)
                    w2_ref[pl.ds(row, 8), pl.ds(c0, DH)] = lo
                    w2_ref[pl.ds(row, 8), pl.ds(c1, DH)] = hi

        for c in in_copies(0):
            c.start()
        kpad_ref[pl.ds(0, 8), :] = jnp.zeros((8, CC), F32)

        def start_w(cc):
            for m in range(3):
                for i in range(cpg):
                    for c in w_copies(cc, m, i):
                        c.start()

        def chunk(cc, _):
            for c in in_copies(cc):
                c.wait()

            @pl.when(cc == 0)
            def _():
                start_w(cc)

            @pl.when(cc + 1 < n_cc)
            def _():
                for c in in_copies(cc + 1):
                    c.start()

            cs = pl.ds(pl.multiple_of(cc * CC, CC), CC)
            kpad_ref[pl.ds(8, S), :] = k_ref[:, cs].astype(F32)

            def fwd_block(j, _):
                t0 = pl.multiple_of(j * TB, TB)
                acc = None
                win = kpad_ref[pl.ds(t0, TB + 8), :]
                for tap in range(4):
                    w = shift_ref[pl.ds(tap, 1), cs].astype(F32)
                    term = win[8 - tap:8 - tap + TB, :] * w
                    acc = term if acc is None else acc + term
                kvb = (acc * v_ref[pl.ds(t0, TB), cs].astype(F32)).astype(BF16)
                kv_ref[pl.ds(t0, TB), :] = kvb
                uh_ref[j] = _nn(fwd_ref[...], kvb)
                kh_ref[j] = _nt(fwd_ref[...], ssmk_ref[cs, pl.ds(t0, TB)])
                return 0

            jax.lax.fori_loop(0, NB // UNR, unrolled(fwd_block), 0)

            for m in range(3):
                for i in range(cpg):
                    for c in w_copies(cc, m, i):
                        c.wait()
                    retile(m, i, cc)

                    @pl.when(cc + 1 < n_cc)
                    def _():
                        for c in w_copies(cc + 1, m, i):
                            c.start()

            @pl.when(cc == WO_AT)
            def _():
                wo_copy.start()

            @pl.when(cc == n_cc - 1)
            def _():
                x_copies[0].start()
                x_copies[1].start()

            sgn = sgn_ref[pl.ds(0, 8), :]

            def spec_tile(ft, _):
                f0 = pl.multiple_of(ft * 8, 8)
                for lc in range(CC // 128):
                    ls = pl.ds(lc * 128, 128)
                    kr0 = [kh_ref[m, pl.ds(f0, 8), ls] for m in range(NB)]
                    ki0 = [kh_ref[m, pl.ds(TB + f0, 8), ls] for m in range(NB)]
                    kr = [kr0[0]] + [kr0[m] - sgn * ki0[m - 1] for m in range(1, NB)]
                    ki = [ki0[0]] + [ki0[m] + sgn * kr0[m - 1] for m in range(1, NB)]
                    ur = [uh_ref[j, pl.ds(f0, 8), ls] for j in range(NB)]
                    ui = [uh_ref[j, pl.ds(TB + f0, 8), ls] for j in range(NB)]
                    for i in range(NB):
                        zr = None
                        zi = None
                        for m in range(i + 1):
                            tr = kr[m] * ur[i - m] - ki[m] * ui[i - m]
                            ti = kr[m] * ui[i - m] + ki[m] * ur[i - m]
                            zr = tr if zr is None else zr + tr
                            zi = ti if zi is None else zi + ti
                        kh_ref[i, pl.ds(f0, 8), ls] = zr
                        kh_ref[i, pl.ds(TB + f0, 8), ls] = zi
                return 0

            jax.lax.fori_loop(0, TB // 8, spec_tile, 0)

            def inv_block(i, _):
                t0 = pl.multiple_of(i * TB, TB)
                yb = _nn(inv_ref[...], kh_ref[i].astype(BF16))
                yb = yb + kv_ref[pl.ds(t0, TB), :].astype(F32) * ssmd_ref[:, cs].astype(F32)
                y_ref[pl.ds(t0, TB), cs] = yb.astype(BF16)
                return 0

            jax.lax.fori_loop(0, NB // UNR, unrolled(inv_block), 0)

            return 0

        jax.lax.fori_loop(0, n_cc, chunk, 0)

        wo_copy.wait()

        def wo_retile(b, _):
            wo2_ref[pl.ds(pl.multiple_of(b * 128, 128), 128), :] = pltpu.bitcast(
                stage_o_ref[pl.ds(pl.multiple_of(b * 256, 256), 256), :], U32)
            return 0

        jax.lax.fori_loop(0, D * 4 // 256, wo_retile, 0)
        x_copies[0].wait()

    pl.run_scoped(
        phase_a,
        pltpu.VMEM((S, D), BF16), pltpu.VMEM((S, D), BF16), pltpu.VMEM((D, S), BF16),
        pltpu.VMEM((S + 8, CC), F32), pltpu.VMEM((S, CC), BF16),
        pltpu.VMEM((NB, 2 * TB, CC), F32), pltpu.VMEM((NB, 2 * TB, CC), F32),
        pltpu.VMEM((6 * (CC // DCH), DCH // 2, WPITCH, DH), U32), pltpu.VMEM((NH * DH, D), BF16),
    )

    scale = DH ** -0.5
    row = jax.lax.broadcasted_iota(jnp.int32, (L, L), 0)
    col = jax.lax.broadcasted_iota(jnp.int32, (L, L), 1)
    mask = (row < MEM) | (row >= col)

    def out_copy(s):
        r = pl.multiple_of(s * SEG, SEG)
        return pltpu.make_async_copy(out_ref.at[pl.ds(r, SEG), :], o_hbm.at[pl.ds(r, SEG), :], sem_out)

    def epilogue(s):
        r = pl.multiple_of(s * SEG, SEG)
        xs = x_ref[pl.ds(r, SEG), :].astype(F32)
        gsum = jnp.sum((xs * gate_ref[...].astype(F32)).astype(BF16).astype(F32), axis=-1, keepdims=True)
        gte = jax.nn.sigmoid(gsum.astype(BF16).astype(F32))
        a = (xs * y_ref[pl.ds(r, SEG), :].astype(F32)).astype(BF16).astype(F32)
        out_ref[pl.ds(r, SEG), :] = (gte * a + (1.0 - gte) * b_ref[...].astype(F32)).astype(BF16)

    def seg_body(s, mem):
        @pl.when(s == XSPLIT // SEG)
        def _():
            x_copies[1].wait()

        r = pl.multiple_of(s * SEG, SEG)
        xs = x_ref[pl.ds(r, SEG), :].astype(F32)
        h = jnp.concatenate([mem, xs], axis=0)
        ngrp = NH // HG
        qkvs = [None] * ngrp
        os_ = [None] * NH

        def attend(g):
            qkv = qkvs[g]
            for hh in range(HG):
                q = qkv[:, (3 * hh) * DH:(3 * hh + 1) * DH].astype(BF16).astype(F32)
                k = qkv[:, (3 * hh + 1) * DH:(3 * hh + 2) * DH].astype(BF16)
                v = qkv[:, (3 * hh + 2) * DH:(3 * hh + 3) * DH].astype(BF16)
                sc = _nt(q, k) * scale
                sc = jnp.where(mask, sc, -1e9)
                mx = jnp.max(sc, axis=-1, keepdims=True)
                e = jnp.exp(sc - mx)
                p = e / jnp.sum(e, axis=-1, keepdims=True)
                o = _nn(p.astype(BF16).astype(F32), v)
                os_[g * HG + hh] = o.astype(BF16).astype(F32)

        for g in range(ngrp + LAG):
            if g < ngrp:
                wg = pltpu.bitcast(w2_ref[:, pl.ds(g * HG * 3 * DH, HG * 3 * DH)], BF16)
                qkvs[g] = _nn(h, wg)
            if g == EPI:
                epilogue(jnp.maximum(s - 1, 0))
            if g >= LAG and g - LAG < ngrp - TAIL:
                attend(g - LAG)
        acc = None
        nwo = NH // WOG
        for g in range(nwo):
            if g == nwo - 1 - TAILPOS:
                for t in range(ngrp - TAIL, ngrp):
                    attend(t)
            og = jnp.concatenate(os_[g * WOG:(g + 1) * WOG], axis=1)
            wog = pltpu.bitcast(wo2_ref[pl.ds(g * WOG * DH // 2, WOG * DH // 2), :], BF16)
            part = _nn(og, wog)
            acc = part if acc is None else acc + part
        ob = acc.astype(BF16)
        b_ref[...] = ob[MEM:]

        @pl.when(s > 0)
        def _():
            out_copy(s - 1).start()

        return ob[:MEM].astype(F32)

    b_ref[...] = jnp.zeros((SEG, D), BF16)
    jax.lax.fori_loop(0, NSEG, seg_body, mem0_ref[...].astype(F32))
    epilogue(NSEG - 1)
    out_copy(NSEG - 1).start()
    pltpu.make_async_copy(out_ref, o_hbm, sem_out).wait()


@functools.partial(jax.jit, static_argnames=("B_seg_len",))
def pallas_gated_mix__ssm_conv_h3__memory_aug_recurrent_mem_tr__prompt_kernel(
    A_q, A_k, A_v, A_shift_k, A_ssm_k, A_ssm_D, B_x, B_mem0, B_Wq, B_Wk, B_Wv, B_Wo, B_seg_len, gate_w,
):
    del B_x
    assert B_seg_len == SEG
    fwd, inv, sgn = _dft_consts()
    any_spec = pl.BlockSpec(memory_space=pl.ANY)
    vmem_spec = pl.BlockSpec(memory_space=pltpu.VMEM)
    out = pl.pallas_call(
        _kernel,
        out_shape=jax.ShapeDtypeStruct((S, D), BF16),
        in_specs=[any_spec] * 8 + [vmem_spec] * 7,
        out_specs=any_spec,
        scratch_shapes=[
            pltpu.VMEM((S, D), BF16),
            pltpu.VMEM((S, D), BF16),
            pltpu.VMEM((D // 2, 3 * NH * DH), U32),
            pltpu.VMEM((NH * DH // 2, D), U32),
            pltpu.VMEM((S, D), BF16),
            pltpu.VMEM((SEG, D), BF16),
            pltpu.SemaphoreType.DMA((3 * (D // CC) + 1,)),
            pltpu.SemaphoreType.DMA((6 * (CC // DCH) + 1,)),
            pltpu.SemaphoreType.DMA((2,)),
            pltpu.SemaphoreType.DMA(()),
        ],
        compiler_params=pltpu.CompilerParams(vmem_limit_bytes=120 * 1024 * 1024),
    )(
        A_q.reshape(S, D), A_k.reshape(S, D), A_v.reshape(S, D), A_ssm_k,
        B_Wq.reshape(D // 2, 2 * NH, DH), B_Wk.reshape(D // 2, 2 * NH, DH), B_Wv.reshape(D // 2, 2 * NH, DH),
        B_Wo.reshape(NH * DH, D),
        A_shift_k.T, A_ssm_D.reshape(1, D), gate_w.reshape(1, D), B_mem0.reshape(MEM, D),
        jnp.asarray(fwd.astype(jnp.bfloat16)), jnp.asarray(inv.astype(jnp.bfloat16)), jnp.asarray(sgn),
    )
    return out.reshape(1, S, D)
```

```python
import functools

import numpy as np
import jax
import jax.numpy as jnp
import jax.experimental.pallas as pl
import jax.experimental.pallas.tpu as pltpu

F32 = jnp.float32
BF16 = jnp.bfloat16
U32 = jnp.uint32

S = 2048
D = 1024
NH = 32
DH = 128
MEM = 8
SEG = 32
NSEG = S // SEG
L = MEM + SEG

TB = 256
NB = S // TB
CC = 256
DCH = 128
WPITCH = 24
WO_AT = 1
XSPLIT = 128
UNR = 4
L1 = 2
L2 = 5
WOG = 4
TOFF = 1
TRATE = 1
SUNR = 1


def _dft_consts():
    n = 2 * TB
    t = np.arange(TB, dtype=np.float64)[None, :]
    f = (np.arange(TB, dtype=np.float64) + 0.5)[:, None]
    ang = 2.0 * np.pi * t * f / n
    fwd = np.concatenate([np.cos(ang), -np.sin(ang)], axis=0)
    inv = np.concatenate([np.cos(ang).T, -np.sin(ang).T], axis=1) * (2.0 / n)
    sgn = np.where(np.arange(TB) % 2 == 0, 1.0, -1.0)[:, None] * np.ones((1, 128))
    return fwd.astype(np.float32), inv.astype(np.float32), sgn.astype(np.float32)


def _nt(a, b):
    return jax.lax.dot_general(a, b, (((1,), (1,)), ((), ())), preferred_element_type=F32)


def _nn(a, b):
    return jax.lax.dot_general(a, b, (((1,), (0,)), ((), ())), preferred_element_type=F32)


def unrolled(body):
    def run(j, c):
        for u in range(UNR):
            body(UNR * j + u, c)
        return c
    return run


def _kernel(xq_hbm, k_hbm, v_hbm, ssmk_hbm, wq_hbm, wk_hbm, wv_hbm, wo_hbm,
            shift_ref, ssmd_ref, gate_ref, mem0_ref, fwd_ref, inv_ref, sgn_ref,
            o_hbm,
            x_ref, y_ref, w2_ref, wo2_ref, out_ref, sem_in, sem_w, sem_x, sem_out):
    x_copies = [
        pltpu.make_async_copy(xq_hbm.at[pl.ds(0, XSPLIT), :], x_ref.at[pl.ds(0, XSPLIT), :], sem_x.at[0]),
        pltpu.make_async_copy(xq_hbm.at[pl.ds(XSPLIT, S - XSPLIT), :], x_ref.at[pl.ds(XSPLIT, S - XSPLIT), :],
                              sem_x.at[1]),
    ]

    def phase_a(k_ref, v_ref, ssmk_ref, kpad_ref, kv_ref, uh_ref, kh_ref, stage_ref, stage_o_ref):
        n_cc = D // CC
        w_hbms = (wq_hbm, wk_hbm, wv_hbm)
        cpg = D // DCH // n_cc

        def in_copies(cc):
            c0 = pl.multiple_of(cc * CC, CC)
            return (
                pltpu.make_async_copy(k_hbm.at[:, pl.ds(c0, CC)], k_ref.at[:, pl.ds(c0, CC)], sem_in.at[3 * cc]),
                pltpu.make_async_copy(v_hbm.at[:, pl.ds(c0, CC)], v_ref.at[:, pl.ds(c0, CC)], sem_in.at[3 * cc + 1]),
                pltpu.make_async_copy(ssmk_hbm.at[pl.ds(c0, CC), :], ssmk_ref.at[pl.ds(c0, CC), :],
                                      sem_in.at[3 * cc + 2]),
            )

        def w_copies(cc, m, i):
            src = w_hbms[m].bitcast(U32)
            r0 = pl.multiple_of((cc * cpg + i) * (DCH // 2), DCH // 2)
            job = m * cpg + i
            return [
                pltpu.make_async_copy(
                    src.at[pl.ds(r0, DCH // 2), pl.ds(par * (NH // 2), NH // 2), :],
                    stage_ref.at[2 * job + par, :, pl.ds(0, NH // 2), :], sem_w.at[2 * job + par])
                for par in range(2)
            ]

        wo_copy = pltpu.make_async_copy(wo_hbm, stage_o_ref, sem_w.at[6 * cpg])

        def retile(m, i, cc):
            jj = m * cpg + i
            c = cc * cpg + i
            ev_ref = stage_ref.at[2 * jj].reshape(DCH // 2 * WPITCH, DH)
            od_ref = stage_ref.at[2 * jj + 1].reshape(DCH // 2 * WPITCH, DH)
            for j in range(NH // 2):
                c0 = pl.multiple_of((2 * j * 3 + m) * DH, DH)
                c1 = pl.multiple_of(((2 * j + 1) * 3 + m) * DH, DH)
                for b in range(DCH // 16):
                    r0 = b * 8 * WPITCH + j
                    ev = ev_ref[pl.ds(r0, 8, stride=WPITCH), :]
                    od = od_ref[pl.ds(r0, 8, stride=WPITCH), :]
                    lo = (ev & jnp.uint32(0xFFFF)) | (od << 16)
                    hi = (ev >> 16) | (od & jnp.uint32(0xFFFF0000))
                    row = pl.multiple_of(c * (DCH // 2) + 8 * b, 8)
                    w2_ref[pl.ds(row, 8), pl.ds(c0, DH)] = lo
                    w2_ref[pl.ds(row, 8), pl.ds(c1, DH)] = hi

        for c in in_copies(0):
            c.start()
        kpad_ref[pl.ds(0, 8), :] = jnp.zeros((8, CC), F32)

        def start_w(cc):
            for m in range(3):
                for i in range(cpg):
                    for c in w_copies(cc, m, i):
                        c.start()

        def chunk(cc, _):
            for c in in_copies(cc):
                c.wait()

            @pl.when(cc == 0)
            def _():
                start_w(cc)

            @pl.when(cc + 1 < n_cc)
            def _():
                for c in in_copies(cc + 1):
                    c.start()

            cs = pl.ds(pl.multiple_of(cc * CC, CC), CC)
            kpad_ref[pl.ds(8, S), :] = k_ref[:, cs].astype(F32)

            def fwd_block(j, _):
                t0 = pl.multiple_of(j * TB, TB)
                acc = None
                win = kpad_ref[pl.ds(t0, TB + 8), :]
                for tap in range(4):
                    w = shift_ref[pl.ds(tap, 1), cs].astype(F32)
                    term = win[8 - tap:8 - tap + TB, :] * w
                    acc = term if acc is None else acc + term
                kvb = (acc * v_ref[pl.ds(t0, TB), cs].astype(F32)).astype(BF16)
                kv_ref[pl.ds(t0, TB), :] = kvb
                uh_ref[j] = _nn(fwd_ref[...], kvb)
                kh_ref[j] = _nt(fwd_ref[...], ssmk_ref[cs, pl.ds(t0, TB)])
                return 0

            jax.lax.fori_loop(0, NB // UNR, unrolled(fwd_block), 0)

            @pl.when(cc == WO_AT)
            def _():
                wo_copy.start()

            @pl.when(cc == n_cc - 1)
            def _():
                x_copies[0].start()
                x_copies[1].start()

            sgn = sgn_ref[pl.ds(0, 8), :]

            def spec_tile(ft, _):
                f0 = pl.multiple_of(ft * 8, 8)
                for lc in range(CC // 128):
                    ls = pl.ds(lc * 128, 128)
                    kr0 = [kh_ref[m, pl.ds(f0, 8), ls] for m in range(NB)]
                    ki0 = [kh_ref[m, pl.ds(TB + f0, 8), ls] for m in range(NB)]
                    kr = [kr0[0]] + [kr0[m] - sgn * ki0[m - 1] for m in range(1, NB)]
                    ki = [ki0[0]] + [ki0[m] + sgn * kr0[m - 1] for m in range(1, NB)]
                    ur = [uh_ref[j, pl.ds(f0, 8), ls] for j in range(NB)]
                    ui = [uh_ref[j, pl.ds(TB + f0, 8), ls] for j in range(NB)]
                    for i in range(NB):
                        zr = None
                        zi = None
                        for m in range(i + 1):
                            tr = kr[m] * ur[i - m] - ki[m] * ui[i - m]
                            ti = kr[m] * ui[i - m] + ki[m] * ur[i - m]
                            zr = tr if zr is None else zr + tr
                            zi = ti if zi is None else zi + ti
                        kh_ref[i, pl.ds(f0, 8), ls] = zr
                        kh_ref[i, pl.ds(TB + f0, 8), ls] = zi
                return 0

            jax.lax.fori_loop(0, TB // 8, spec_tile, 0)

            def inv_block(i, _):
                t0 = pl.multiple_of(i * TB, TB)
                yb = _nn(inv_ref[...], kh_ref[i].astype(BF16))
                yb = yb + kv_ref[pl.ds(t0, TB), :].astype(F32) * ssmd_ref[:, cs].astype(F32)
                y_ref[pl.ds(t0, TB), cs] = yb.astype(BF16)
                return 0

            jax.lax.fori_loop(0, NB // UNR, unrolled(inv_block), 0)

            for m in range(3):
                for i in range(cpg):
                    for c in w_copies(cc, m, i):
                        c.wait()
                    retile(m, i, cc)

                    @pl.when(cc + 1 < n_cc)
                    def _():
                        for c in w_copies(cc + 1, m, i):
                            c.start()

            return 0

        jax.lax.fori_loop(0, n_cc, chunk, 0)

        wo_copy.wait()

        def wo_retile(b, _):
            wo2_ref[pl.ds(pl.multiple_of(b * 128, 128), 128), :] = pltpu.bitcast(
                stage_o_ref[pl.ds(pl.multiple_of(b * 256, 256), 256), :], U32)
            return 0

        jax.lax.fori_loop(0, D * 4 // 256, wo_retile, 0)
        x_copies[0].wait()

    pl.run_scoped(
        phase_a,
        pltpu.VMEM((S, D), BF16), pltpu.VMEM((S, D), BF16), pltpu.VMEM((D, S), BF16),
        pltpu.VMEM((S + 8, CC), F32), pltpu.VMEM((S, CC), BF16),
        pltpu.VMEM((NB, 2 * TB, CC), F32), pltpu.VMEM((NB, 2 * TB, CC), F32),
        pltpu.VMEM((6 * (CC // DCH), DCH // 2, WPITCH, DH), U32), pltpu.VMEM((NH * DH, D), BF16),
    )

    scale = DH ** -0.5
    row = jax.lax.broadcasted_iota(jnp.int32, (L, L), 0)
    col = jax.lax.broadcasted_iota(jnp.int32, (L, L), 1)
    mask = (row < MEM) | (row >= col)

    def out_copy(t):
        r = pl.multiple_of(t * (SEG * SUNR), SEG * SUNR)
        return pltpu.make_async_copy(out_ref.at[pl.ds(r, SEG * SUNR), :], o_hbm.at[pl.ds(r, SEG * SUNR), :], sem_out)

    def epilogue(s, b):
        r = pl.multiple_of(s * SEG, SEG)
        xs = x_ref[pl.ds(r, SEG), :].astype(F32)
        gsum = jnp.sum((xs * gate_ref[...].astype(F32)).astype(BF16).astype(F32), axis=-1, keepdims=True)
        gte = jax.nn.sigmoid(gsum.astype(BF16).astype(F32))
        a = (xs * y_ref[pl.ds(r, SEG), :].astype(F32)).astype(BF16).astype(F32)
        out_ref[pl.ds(r, SEG), :] = (gte * a + (1.0 - gte) * b.astype(F32)).astype(BF16)

    def seg_body(s, mem):
        r = pl.multiple_of(s * SEG, SEG)
        xs = x_ref[pl.ds(r, SEG), :].astype(F32)
        h = jnp.concatenate([mem, xs], axis=0)
        qkvs = [None] * NH
        ps = [None] * NH
        os_ = [None] * NH

        def probs(hd):
            q = qkvs[hd][:, 0:DH].astype(BF16).astype(F32)
            k = qkvs[hd][:, DH:2 * DH].astype(BF16)
            sc = jnp.where(mask, _nt(q, k) * scale, -1e9)
            e = jnp.exp(sc - jnp.max(sc, axis=-1, keepdims=True))
            ps[hd] = (e / jnp.sum(e, axis=-1, keepdims=True)).astype(BF16).astype(F32)

        def values(hd):
            o = _nn(ps[hd], qkvs[hd][:, 2 * DH:3 * DH].astype(BF16))
            os_[hd] = o.astype(BF16).astype(F32)

        def slot(g):
            if g < NH:
                qkvs[g] = _nn(h, pltpu.bitcast(w2_ref[:, pl.ds(g * 3 * DH, 3 * DH)], BF16))
            if 0 <= g - L1 < NH:
                probs(g - L1)
            if 0 <= g - L2 < NH:
                values(g - L2)

        for g in range(NH):
            slot(g)
        acc = None
        nxt = NH
        for w in range(NH // WOG):
            while nxt < NH + L2 and (nxt - NH < (w + 1 - TOFF) * TRATE or nxt - L2 < (w + 1) * WOG):
                slot(nxt)
                nxt += 1
            og = jnp.concatenate(os_[w * WOG:(w + 1) * WOG], axis=1)
            wog = pltpu.bitcast(wo2_ref[pl.ds(w * WOG * DH // 2, WOG * DH // 2), :], BF16)
            part = _nn(og, wog)
            acc = part if acc is None else acc + part
        ob = acc.astype(BF16)
        epilogue(s, ob[MEM:])
        return ob[:MEM].astype(F32)

    def seg_pair(t, mem):
        @pl.when(t == XSPLIT // (SEG * SUNR))
        def _():
            x_copies[1].wait()

        for u in range(SUNR):
            mem = seg_body(t * SUNR + u, mem)
        out_copy(t).start()
        return mem

    jax.lax.fori_loop(0, NSEG // SUNR, seg_pair, mem0_ref[...].astype(F32))
    pltpu.make_async_copy(out_ref, o_hbm, sem_out).wait()


@functools.partial(jax.jit, static_argnames=("B_seg_len",))
def pallas_gated_mix__ssm_conv_h3__memory_aug_recurrent_mem_tr__prompt_kernel(
    A_q, A_k, A_v, A_shift_k, A_ssm_k, A_ssm_D, B_x, B_mem0, B_Wq, B_Wk, B_Wv, B_Wo, B_seg_len, gate_w,
):
    del B_x
    assert B_seg_len == SEG
    fwd, inv, sgn = _dft_consts()
    any_spec = pl.BlockSpec(memory_space=pl.ANY)
    vmem_spec = pl.BlockSpec(memory_space=pltpu.VMEM)
    out = pl.pallas_call(
        _kernel,
        out_shape=jax.ShapeDtypeStruct((S, D), BF16),
        in_specs=[any_spec] * 8 + [vmem_spec] * 7,
        out_specs=any_spec,
        scratch_shapes=[
            pltpu.VMEM((S, D), BF16),
            pltpu.VMEM((S, D), BF16),
            pltpu.VMEM((D // 2, 3 * NH * DH), U32),
            pltpu.VMEM((NH * DH // 2, D), U32),
            pltpu.VMEM((S, D), BF16),
            pltpu.SemaphoreType.DMA((3 * (D // CC) + 1,)),
            pltpu.SemaphoreType.DMA((6 * (CC // DCH) + 1,)),
            pltpu.SemaphoreType.DMA((2,)),
            pltpu.SemaphoreType.DMA(()),
        ],
        compiler_params=pltpu.CompilerParams(vmem_limit_bytes=120 * 1024 * 1024),
    )(
        A_q.reshape(S, D), A_k.reshape(S, D), A_v.reshape(S, D), A_ssm_k,
        B_Wq.reshape(D // 2, 2 * NH, DH), B_Wk.reshape(D // 2, 2 * NH, DH), B_Wv.reshape(D // 2, 2 * NH, DH),
        B_Wo.reshape(NH * DH, D),
        A_shift_k.T, A_ssm_D.reshape(1, D), gate_w.reshape(1, D), B_mem0.reshape(MEM, D),
        jnp.asarray(fwd.astype(jnp.bfloat16)), jnp.asarray(inv.astype(jnp.bfloat16)), jnp.asarray(sgn),
    )
    return out.reshape(1, S, D)
```

```python
import functools

import numpy as np
import jax
import jax.numpy as jnp
import jax.experimental.pallas as pl
import jax.experimental.pallas.tpu as pltpu

F32 = jnp.float32
BF16 = jnp.bfloat16
U32 = jnp.uint32

S = 2048
D = 1024
NH = 32
DH = 128
MEM = 8
SEG = 32
NSEG = S // SEG
L = MEM + SEG

TB = 256
NB = S // TB
CC = 256
DCH = 128
WPITCH = 24
XSPLIT = 128
UNR = 4
L1 = 2
L2 = 5
WOG = 4
TOFF = 1
TRATE = 1
SUNR = 2


def _dft_consts():
    n = 2 * TB
    t = np.arange(TB, dtype=np.float64)[None, :]
    f = (np.arange(TB, dtype=np.float64) + 0.5)[:, None]
    ang = 2.0 * np.pi * t * f / n
    fwd = np.concatenate([np.cos(ang), -np.sin(ang)], axis=0)
    inv = np.concatenate([np.cos(ang).T, -np.sin(ang).T], axis=1) * (2.0 / n)
    sgn = np.where(np.arange(TB) % 2 == 0, 1.0, -1.0)[:, None] * np.ones((1, 128))
    return fwd.astype(np.float32), inv.astype(np.float32), sgn.astype(np.float32)


def _nt(a, b):
    return jax.lax.dot_general(a, b, (((1,), (1,)), ((), ())), preferred_element_type=F32)


def _nn(a, b):
    return jax.lax.dot_general(a, b, (((1,), (0,)), ((), ())), preferred_element_type=F32)


def unrolled(body):
    def run(j, c):
        for u in range(UNR):
            body(UNR * j + u, c)
        return c
    return run


def _kernel(xq_hbm, k_hbm, v_hbm, ssmk_hbm, wq_hbm, wk_hbm, wv_hbm, wo_hbm,
            shift_ref, ssmd_ref, gate_ref, mem0_ref, fwd_ref, inv_ref, sgn_ref,
            o_hbm,
            x_ref, y_ref, w2_ref, wo2_ref, out_ref, sem_in, sem_w, sem_x, sem_out):
    x_copies = [
        pltpu.make_async_copy(xq_hbm.at[pl.ds(0, XSPLIT), :], x_ref.at[pl.ds(0, XSPLIT), :], sem_x.at[0]),
        pltpu.make_async_copy(xq_hbm.at[pl.ds(XSPLIT, S - XSPLIT), :], x_ref.at[pl.ds(XSPLIT, S - XSPLIT), :],
                              sem_x.at[1]),
    ]

    def phase_a(k_ref, v_ref, ssmk_ref, kpad_ref, kv_ref, uh_ref, kh_ref, stage_ref, stage_o_ref):
        n_cc = D // CC
        w_hbms = (wq_hbm, wk_hbm, wv_hbm)
        cpg = D // DCH // n_cc

        def filt_copy(cc):
            c0 = pl.multiple_of(cc * CC, CC)
            return pltpu.make_async_copy(ssmk_hbm.at[pl.ds(c0, CC), :], ssmk_ref.at[pl.ds(c0, CC), :],
                                         sem_in.at[3 * cc + 2])

        def in_copies(cc):
            c0 = pl.multiple_of(cc * CC, CC)
            return (
                pltpu.make_async_copy(k_hbm.at[:, pl.ds(c0, CC)], k_ref.at[:, pl.ds(c0, CC)], sem_in.at[3 * cc]),
                pltpu.make_async_copy(v_hbm.at[:, pl.ds(c0, CC)], v_ref.at[:, pl.ds(c0, CC)], sem_in.at[3 * cc + 1]),
                filt_copy(cc),
            )

        def w_copies(cc, m, i):
            src = w_hbms[m].bitcast(U32)
            r0 = pl.multiple_of((cc * cpg + i) * (DCH // 2), DCH // 2)
            job = m * cpg + i
            return [
                pltpu.make_async_copy(
                    src.at[pl.ds(r0, DCH // 2), pl.ds(par * (NH // 2), NH // 2), :],
                    stage_ref.at[2 * job + par, :, pl.ds(0, NH // 2), :], sem_w.at[2 * job + par])
                for par in range(2)
            ]

        wo_rows = NH * DH // n_cc

        def wo_copy(cc):
            r0 = pl.multiple_of(cc * wo_rows, wo_rows)
            return pltpu.make_async_copy(wo_hbm.at[pl.ds(r0, wo_rows), :], stage_o_ref.at[pl.ds(r0, wo_rows), :],
                                         sem_w.at[6 * cpg + cc])

        def wo_retile(cc):
            wo_copy(cc).wait()
            for b in range(wo_rows // 256):
                r0 = pl.multiple_of(cc * wo_rows + b * 256, 256)
                wo2_ref[pl.ds(pl.multiple_of(r0 // 2, 128), 128), :] = pltpu.bitcast(
                    stage_o_ref[pl.ds(r0, 256), :], U32)

        def retile(m, i, cc):
            jj = m * cpg + i
            c = cc * cpg + i
            ev_ref = stage_ref.at[2 * jj].reshape(DCH // 2 * WPITCH, DH)
            od_ref = stage_ref.at[2 * jj + 1].reshape(DCH // 2 * WPITCH, DH)
            for j in range(NH // 2):
                c0 = pl.multiple_of((2 * j * 3 + m) * DH, DH)
                c1 = pl.multiple_of(((2 * j + 1) * 3 + m) * DH, DH)
                for b in range(DCH // 16):
                    r0 = b * 8 * WPITCH + j
                    ev = ev_ref[pl.ds(r0, 8, stride=WPITCH), :]
                    od = od_ref[pl.ds(r0, 8, stride=WPITCH), :]
                    lo = (ev & jnp.uint32(0xFFFF)) | (od << 16)
                    hi = (ev >> 16) | (od & jnp.uint32(0xFFFF0000))
                    row = pl.multiple_of(c * (DCH // 2) + 8 * b, 8)
                    w2_ref[pl.ds(row, 8), pl.ds(c0, DH)] = lo
                    w2_ref[pl.ds(row, 8), pl.ds(c1, DH)] = hi

        filt_copy(0).start()
        kpad_ref[pl.ds(0, 8), :] = jnp.zeros((8, CC), F32)

        def start_w(cc):
            for m in range(3):
                for i in range(cpg):
                    for c in w_copies(cc, m, i):
                        c.start()

        def chunk(cc, _):
            cur = in_copies(cc)
            cur[2].wait()

            @pl.when(cc == 0)
            def _():
                cur[0].start()
                cur[1].start()

            cs = pl.ds(pl.multiple_of(cc * CC, CC), CC)

            def filt_block(j, _):
                t0 = pl.multiple_of(j * TB, TB)
                kh_ref[j] = _nt(fwd_ref[...], ssmk_ref[cs, pl.ds(t0, TB)])
                return 0

            jax.lax.fori_loop(0, NB // UNR, unrolled(filt_block), 0)
            cur[0].wait()
            cur[1].wait()

            @pl.when(cc == 0)
            def _():
                start_w(cc)

            @pl.when(cc + 1 < n_cc)
            def _():
                for c in in_copies(cc + 1):
                    c.start()
            wo_copy(cc).start()

            kpad_ref[pl.ds(8, S), :] = k_ref[:, cs].astype(F32)

            def fwd_block(j, _):
                t0 = pl.multiple_of(j * TB, TB)
                acc = None
                win = kpad_ref[pl.ds(t0, TB + 8), :]
                for tap in range(4):
                    w = shift_ref[pl.ds(tap, 1), cs].astype(F32)
                    term = win[8 - tap:8 - tap + TB, :] * w
                    acc = term if acc is None else acc + term
                kvb = (acc * v_ref[pl.ds(t0, TB), cs].astype(F32)).astype(BF16)
                kv_ref[pl.ds(t0, TB), :] = kvb
                uh_ref[j] = _nn(fwd_ref[...], kvb)
                return 0

            jax.lax.fori_loop(0, NB // UNR, unrolled(fwd_block), 0)

            @pl.when(cc > 0)
            def _():
                wo_retile(cc - 1)

            @pl.when(cc == n_cc - 1)
            def _():
                x_copies[0].start()
                x_copies[1].start()

            sgn = sgn_ref[pl.ds(0, 8), :]

            def spec_tile(ft, _):
                f0 = pl.multiple_of(ft * 8, 8)
                for lc in range(CC // 128):
                    ls = pl.ds(lc * 128, 128)
                    kr0 = [kh_ref[m, pl.ds(f0, 8), ls] for m in range(NB)]
                    ki0 = [kh_ref[m, pl.ds(TB + f0, 8), ls] for m in range(NB)]
                    kr = [kr0[0]] + [kr0[m] - sgn * ki0[m - 1] for m in range(1, NB)]
                    ki = [ki0[0]] + [ki0[m] + sgn * kr0[m - 1] for m in range(1, NB)]
                    ur = [uh_ref[j, pl.ds(f0, 8), ls] for j in range(NB)]
                    ui = [uh_ref[j, pl.ds(TB + f0, 8), ls] for j in range(NB)]
                    for i in range(NB):
                        zr = None
                        zi = None
                        for m in range(i + 1):
                            tr = kr[m] * ur[i - m] - ki[m] * ui[i - m]
                            ti = kr[m] * ui[i - m] + ki[m] * ur[i - m]
                            zr = tr if zr is None else zr + tr
                            zi = ti if zi is None else zi + ti
                        kh_ref[i, pl.ds(f0, 8), ls] = zr
                        kh_ref[i, pl.ds(TB + f0, 8), ls] = zi
                return 0

            jax.lax.fori_loop(0, TB // 8, spec_tile, 0)

            def inv_block(i, _):
                t0 = pl.multiple_of(i * TB, TB)
                yb = _nn(inv_ref[...], kh_ref[i].astype(BF16))
                yb = yb + kv_ref[pl.ds(t0, TB), :].astype(F32) * ssmd_ref[:, cs].astype(F32)
                y_ref[pl.ds(t0, TB), cs] = yb.astype(BF16)
                return 0

            jax.lax.fori_loop(0, NB // UNR, unrolled(inv_block), 0)

            for m in range(3):
                for i in range(cpg):
                    for c in w_copies(cc, m, i):
                        c.wait()
                    retile(m, i, cc)

                    @pl.when(cc + 1 < n_cc)
                    def _():
                        for c in w_copies(cc + 1, m, i):
                            c.start()

            return 0

        jax.lax.fori_loop(0, n_cc, chunk, 0)

        wo_retile(n_cc - 1)
        x_copies[0].wait()

    pl.run_scoped(
        phase_a,
        pltpu.VMEM((S, D), BF16), pltpu.VMEM((S, D), BF16), pltpu.VMEM((D, S), BF16),
        pltpu.VMEM((S + 8, CC), F32), pltpu.VMEM((S, CC), BF16),
        pltpu.VMEM((NB, 2 * TB, CC), F32), pltpu.VMEM((NB, 2 * TB, CC), F32),
        pltpu.VMEM((6 * (CC // DCH), DCH // 2, WPITCH, DH), U32), pltpu.VMEM((NH * DH, D), BF16),
    )

    scale = DH ** -0.5
    row = jax.lax.broadcasted_iota(jnp.int32, (L, L), 0)
    col = jax.lax.broadcasted_iota(jnp.int32, (L, L), 1)
    mask = (row < MEM) | (row >= col)

    def out_copy(t):
        r = pl.multiple_of(t * (SEG * SUNR), SEG * SUNR)
        return pltpu.make_async_copy(out_ref.at[pl.ds(r, SEG * SUNR), :], o_hbm.at[pl.ds(r, SEG * SUNR), :], sem_out)

    def epilogue(s, b):
        r = pl.multiple_of(s * SEG, SEG)
        xs = x_ref[pl.ds(r, SEG), :].astype(F32)
        gsum = jnp.sum((xs * gate_ref[...].astype(F32)).astype(BF16).astype(F32), axis=-1, keepdims=True)
        gte = jax.nn.sigmoid(gsum.astype(BF16).astype(F32))
        a = (xs * y_ref[pl.ds(r, SEG), :].astype(F32)).astype(BF16).astype(F32)
        out_ref[pl.ds(r, SEG), :] = (gte * a + (1.0 - gte) * b.astype(F32)).astype(BF16)

    def seg_body(s, mem):
        r = pl.multiple_of(s * SEG, SEG)
        xs = x_ref[pl.ds(r, SEG), :].astype(F32)
        h = jnp.concatenate([mem, xs], axis=0)
        qkvs = [None] * NH
        ps = [None] * NH
        os_ = [None] * NH

        def probs(hd):
            q = qkvs[hd][:, 0:DH].astype(BF16).astype(F32)
            k = qkvs[hd][:, DH:2 * DH].astype(BF16)
            sc = jnp.where(mask, _nt(q, k) * scale, -1e9)
            e = jnp.exp(sc - jnp.max(sc, axis=-1, keepdims=True))
            ps[hd] = (e / jnp.sum(e, axis=-1, keepdims=True)).astype(BF16).astype(F32)

        def values(hd):
            o = _nn(ps[hd], qkvs[hd][:, 2 * DH:3 * DH].astype(BF16))
            os_[hd] = o.astype(BF16).astype(F32)

        def slot(g):
            if g < NH:
                qkvs[g] = _nn(h, pltpu.bitcast(w2_ref[:, pl.ds(g * 3 * DH, 3 * DH)], BF16))
            if 0 <= g - L1 < NH:
                probs(g - L1)
            if 0 <= g - L2 < NH:
                values(g - L2)

        for g in range(NH):
            slot(g)
        acc = None
        nxt = NH
        for w in range(NH // WOG):
            while nxt < NH + L2 and (nxt - NH < (w + 1 - TOFF) * TRATE or nxt - L2 < (w + 1) * WOG):
                slot(nxt)
                nxt += 1
            og = jnp.concatenate(os_[w * WOG:(w + 1) * WOG], axis=1)
            wog = pltpu.bitcast(wo2_ref[pl.ds(w * WOG * DH // 2, WOG * DH // 2), :], BF16)
            part = _nn(og, wog)
            acc = part if acc is None else acc + part
        ob = acc.astype(BF16)
        epilogue(s, ob[MEM:])
        return ob[:MEM].astype(F32)

    def seg_pair(t, mem):
        @pl.when(t == XSPLIT // (SEG * SUNR))
        def _():
            x_copies[1].wait()

        for u in range(SUNR):
            mem = seg_body(t * SUNR + u, mem)
        out_copy(t).start()
        return mem

    jax.lax.fori_loop(0, NSEG // SUNR, seg_pair, mem0_ref[...].astype(F32))
    pltpu.make_async_copy(out_ref, o_hbm, sem_out).wait()


@functools.partial(jax.jit, static_argnames=("B_seg_len",))
def pallas_gated_mix__ssm_conv_h3__memory_aug_recurrent_mem_tr__prompt_kernel(
    A_q, A_k, A_v, A_shift_k, A_ssm_k, A_ssm_D, B_x, B_mem0, B_Wq, B_Wk, B_Wv, B_Wo, B_seg_len, gate_w,
):
    del B_x
    assert B_seg_len == SEG
    fwd, inv, sgn = _dft_consts()
    any_spec = pl.BlockSpec(memory_space=pl.ANY)
    vmem_spec = pl.BlockSpec(memory_space=pltpu.VMEM)
    out = pl.pallas_call(
        _kernel,
        out_shape=jax.ShapeDtypeStruct((S, D), BF16),
        in_specs=[any_spec] * 8 + [vmem_spec] * 7,
        out_specs=any_spec,
        scratch_shapes=[
            pltpu.VMEM((S, D), BF16),
            pltpu.VMEM((S, D), BF16),
            pltpu.VMEM((D // 2, 3 * NH * DH), U32),
            pltpu.VMEM((NH * DH // 2, D), U32),
            pltpu.VMEM((S, D), BF16),
            pltpu.SemaphoreType.DMA((3 * (D // CC) + 1,)),
            pltpu.SemaphoreType.DMA((6 * (CC // DCH) + D // CC,)),
            pltpu.SemaphoreType.DMA((2,)),
            pltpu.SemaphoreType.DMA(()),
        ],
        compiler_params=pltpu.CompilerParams(vmem_limit_bytes=120 * 1024 * 1024),
    )(
        A_q.reshape(S, D), A_k.reshape(S, D), A_v.reshape(S, D), A_ssm_k,
        B_Wq.reshape(D // 2, 2 * NH, DH), B_Wk.reshape(D // 2, 2 * NH, DH), B_Wv.reshape(D // 2, 2 * NH, DH),
        B_Wo.reshape(NH * DH, D),
        A_shift_k.T, A_ssm_D.reshape(1, D), gate_w.reshape(1, D), B_mem0.reshape(MEM, D),
        jnp.asarray(fwd.astype(jnp.bfloat16)), jnp.asarray(inv.astype(jnp.bfloat16)), jnp.asarray(sgn),
    )
    return out.reshape(1, S, D)
```

```python
import functools

import numpy as np
import jax
import jax.numpy as jnp
import jax.experimental.pallas as pl
import jax.experimental.pallas.tpu as pltpu

F32 = jnp.float32
BF16 = jnp.bfloat16
U32 = jnp.uint32

S = 2048
D = 1024
NH = 32
DH = 128
MEM = 8
SEG = 32
NSEG = S // SEG
L = MEM + SEG

TB = 256
NB = S // TB
CC = 256
DCH = 128
WPITCH = 24
XSPLIT = 128
UNR = 4
KPAD = 16
L1 = 2
L2 = 5
WOG = 4
TOFF = 1
TRATE = 1
SUNR = 2


def _dft_consts():
    n = 2 * TB
    t = np.arange(TB, dtype=np.float64)[None, :]
    f = (np.arange(TB, dtype=np.float64) + 0.5)[:, None]
    ang = 2.0 * np.pi * t * f / n
    fwd = np.concatenate([np.cos(ang), -np.sin(ang)], axis=0)
    inv = np.concatenate([np.cos(ang).T, -np.sin(ang).T], axis=1) * (2.0 / n)
    sgn = np.where(np.arange(8) % 2 == 0, 1.0, -1.0)[:, None] * np.ones((1, 128))
    return fwd.astype(np.float32), inv.astype(np.float32), sgn.astype(np.float32)


def _nt(a, b):
    return jax.lax.dot_general(a, b, (((1,), (1,)), ((), ())), preferred_element_type=F32)


def _nn(a, b):
    return jax.lax.dot_general(a, b, (((1,), (0,)), ((), ())), preferred_element_type=F32)


def unrolled(body):
    def run(j, c):
        for u in range(UNR):
            body(UNR * j + u, c)
        return c
    return run


def _kernel(xq_hbm, k_hbm, v_hbm, ssmk_hbm, wq_hbm, wk_hbm, wv_hbm, wo_hbm,
            shift_ref, ssmd_ref, gate_ref, mem0_ref, fwd_ref, inv_ref, sgn_ref,
            o_hbm,
            x_ref, y_ref, w2_ref, wo2_ref, out_ref, sem_in, sem_w, sem_x, sem_out):
    x_copies = [
        pltpu.make_async_copy(xq_hbm.at[pl.ds(0, XSPLIT), :], x_ref.at[pl.ds(0, XSPLIT), :], sem_x.at[0]),
        pltpu.make_async_copy(xq_hbm.at[pl.ds(XSPLIT, S - XSPLIT), :], x_ref.at[pl.ds(XSPLIT, S - XSPLIT), :],
                              sem_x.at[1]),
    ]

    def phase_a(k_ref, v_ref, ssmk_ref, kv_ref, uh_ref, kh_ref, stage_ref, stage_o_ref):
        n_cc = D // CC
        w_hbms = (wq_hbm, wk_hbm, wv_hbm)
        cpg = D // DCH // n_cc

        def filt_copy(cc):
            c0 = pl.multiple_of(cc * CC, CC)
            return pltpu.make_async_copy(ssmk_hbm.at[pl.ds(c0, CC), :], ssmk_ref.at[pl.ds(c0, CC), :],
                                         sem_in.at[3 * cc + 2])

        def in_copies(cc):
            c0 = pl.multiple_of(cc * CC, CC)
            return (
                pltpu.make_async_copy(k_hbm.at[:, pl.ds(c0, CC)], k_ref.at[pl.ds(KPAD, S), pl.ds(c0, CC)], sem_in.at[3 * cc]),
                pltpu.make_async_copy(v_hbm.at[:, pl.ds(c0, CC)], v_ref.at[:, pl.ds(c0, CC)], sem_in.at[3 * cc + 1]),
                filt_copy(cc),
            )

        def w_copies(cc, m, i):
            src = w_hbms[m].bitcast(U32)
            r0 = pl.multiple_of((cc * cpg + i) * (DCH // 2), DCH // 2)
            job = m * cpg + i
            return [
                pltpu.make_async_copy(
                    src.at[pl.ds(r0, DCH // 2), pl.ds(par * (NH // 2), NH // 2), :],
                    stage_ref.at[2 * job + par, :, pl.ds(0, NH // 2), :], sem_w.at[2 * job + par])
                for par in range(2)
            ]

        wo_rows = NH * DH // n_cc

        def wo_copy(cc):
            r0 = pl.multiple_of(cc * wo_rows, wo_rows)
            return pltpu.make_async_copy(wo_hbm.at[pl.ds(r0, wo_rows), :], stage_o_ref.at[pl.ds(r0, wo_rows), :],
                                         sem_w.at[6 * cpg + cc])

        def wo_retile(cc):
            wo_copy(cc).wait()
            for b in range(wo_rows // 256):
                r0 = pl.multiple_of(cc * wo_rows + b * 256, 256)
                wo2_ref[pl.ds(pl.multiple_of(r0 // 2, 128), 128), :] = pltpu.bitcast(
                    stage_o_ref[pl.ds(r0, 256), :], U32)

        def retile(m, i, cc):
            jj = m * cpg + i
            c = cc * cpg + i
            ev_ref = stage_ref.at[2 * jj].reshape(DCH // 2 * WPITCH, DH)
            od_ref = stage_ref.at[2 * jj + 1].reshape(DCH // 2 * WPITCH, DH)
            for j in range(NH // 2):
                c0 = pl.multiple_of((2 * j * 3 + m) * DH, DH)
                c1 = pl.multiple_of(((2 * j + 1) * 3 + m) * DH, DH)
                for b in range(DCH // 16):
                    r0 = b * 8 * WPITCH + j
                    ev = ev_ref[pl.ds(r0, 8, stride=WPITCH), :]
                    od = od_ref[pl.ds(r0, 8, stride=WPITCH), :]
                    lo = (ev & jnp.uint32(0xFFFF)) | (od << 16)
                    hi = (ev >> 16) | (od & jnp.uint32(0xFFFF0000))
                    row = pl.multiple_of(c * (DCH // 2) + 8 * b, 8)
                    w2_ref[pl.ds(row, 8), pl.ds(c0, DH)] = lo
                    w2_ref[pl.ds(row, 8), pl.ds(c1, DH)] = hi

        filt_copy(0).start()
        k_ref[pl.ds(0, KPAD), :] = jnp.zeros((KPAD, D), BF16)

        def start_w(cc):
            for m in range(3):
                for i in range(cpg):
                    for c in w_copies(cc, m, i):
                        c.start()

        def chunk(cc, _):
            cur = in_copies(cc)
            cur[2].wait()

            @pl.when(cc == 0)
            def _():
                cur[0].start()
                cur[1].start()

            cs = pl.ds(pl.multiple_of(cc * CC, CC), CC)

            def filt_block(j, _):
                t0 = pl.multiple_of(j * TB, TB)
                kh_ref[j] = _nt(fwd_ref[...], ssmk_ref[cs, pl.ds(t0, TB)])
                return 0

            jax.lax.fori_loop(0, NB // UNR, unrolled(filt_block), 0)
            cur[0].wait()
            cur[1].wait()

            @pl.when(cc == 0)
            def _():
                start_w(cc)

            @pl.when(cc + 1 < n_cc)
            def _():
                for c in in_copies(cc + 1):
                    c.start()

            @pl.when(cc > 0)
            def _():
                wo_copy(cc - 1).start()

            @pl.when(cc == n_cc - 1)
            def _():
                wo_copy(cc).start()

            def fwd_block(j, _):
                t0 = pl.multiple_of(j * TB, TB)
                acc = None
                win = k_ref[pl.ds(t0, TB + KPAD), cs].astype(F32)
                for tap in range(4):
                    w = shift_ref[pl.ds(tap, 1), cs].astype(F32)
                    term = win[KPAD - tap:KPAD - tap + TB, :] * w
                    acc = term if acc is None else acc + term
                kvb = (acc * v_ref[pl.ds(t0, TB), cs].astype(F32)).astype(BF16)
                kv_ref[pl.ds(t0, TB), :] = kvb
                uh_ref[j] = _nn(fwd_ref[...], kvb)
                return 0

            jax.lax.fori_loop(0, NB // UNR, unrolled(fwd_block), 0)

            @pl.when(cc > 1)
            def _():
                wo_retile(cc - 2)

            @pl.when(cc == n_cc - 1)
            def _():
                x_copies[0].start()
                x_copies[1].start()

            sgn = sgn_ref[...]

            def spec_tile(ft, _):
                f0 = pl.multiple_of(ft * 8, 8)
                for lc in range(CC // 128):
                    ls = pl.ds(lc * 128, 128)
                    kr0 = [kh_ref[m, pl.ds(f0, 8), ls] for m in range(NB)]
                    ki0 = [kh_ref[m, pl.ds(TB + f0, 8), ls] for m in range(NB)]
                    kr = [kr0[0]] + [kr0[m] - sgn * ki0[m - 1] for m in range(1, NB)]
                    ki = [ki0[0]] + [ki0[m] + sgn * kr0[m - 1] for m in range(1, NB)]
                    ur = [uh_ref[j, pl.ds(f0, 8), ls] for j in range(NB)]
                    ui = [uh_ref[j, pl.ds(TB + f0, 8), ls] for j in range(NB)]
                    for i in range(NB):
                        zr = None
                        zi = None
                        for m in range(i + 1):
                            tr = kr[m] * ur[i - m] - ki[m] * ui[i - m]
                            ti = kr[m] * ui[i - m] + ki[m] * ur[i - m]
                            zr = tr if zr is None else zr + tr
                            zi = ti if zi is None else zi + ti
                        kh_ref[i, pl.ds(f0, 8), ls] = zr
                        kh_ref[i, pl.ds(TB + f0, 8), ls] = zi
                return 0

            jax.lax.fori_loop(0, TB // 8, spec_tile, 0)

            def inv_block(i, _):
                t0 = pl.multiple_of(i * TB, TB)
                yb = _nn(inv_ref[...], kh_ref[i].astype(BF16))
                yb = yb + kv_ref[pl.ds(t0, TB), :].astype(F32) * ssmd_ref[:, cs].astype(F32)
                y_ref[pl.ds(t0, TB), cs] = yb.astype(BF16)
                return 0

            def inv_retile(i, c):
                for m in range(3):
                    for cp in w_copies(cc, m, i):
                        cp.wait()
                unrolled(inv_block)(i, c)
                for m in range(3):
                    retile(m, i, cc)

                @pl.when(cc + 1 < n_cc)
                def _():
                    for m in range(3):
                        for cp in w_copies(cc + 1, m, i):
                            cp.start()

                return c

            assert NB // UNR == cpg
            jax.lax.fori_loop(0, cpg, inv_retile, 0)
            return 0

        jax.lax.fori_loop(0, n_cc, chunk, 0)

        wo_retile(n_cc - 2)
        wo_retile(n_cc - 1)
        x_copies[0].wait()

    pl.run_scoped(
        phase_a,
        pltpu.VMEM((KPAD + S, D), BF16), pltpu.VMEM((S, D), BF16), pltpu.VMEM((D, S), BF16),
        pltpu.VMEM((S, CC), BF16),
        pltpu.VMEM((NB, 2 * TB, CC), F32), pltpu.VMEM((NB, 2 * TB, CC), F32),
        pltpu.VMEM((6 * (CC // DCH), DCH // 2, WPITCH, DH), U32), pltpu.VMEM((NH * DH, D), BF16),
    )

    scale = DH ** -0.5
    row = jax.lax.broadcasted_iota(jnp.int32, (L, L), 0)
    col = jax.lax.broadcasted_iota(jnp.int32, (L, L), 1)
    mask = (row < MEM) | (row >= col)

    def out_copy(t):
        r = pl.multiple_of(t * (SEG * SUNR), SEG * SUNR)
        return pltpu.make_async_copy(out_ref.at[pl.ds(r, SEG * SUNR), :], o_hbm.at[pl.ds(r, SEG * SUNR), :], sem_out)

    def epilogue(s, b):
        r = pl.multiple_of(s * SEG, SEG)
        xs = x_ref[pl.ds(r, SEG), :].astype(F32)
        gsum = jnp.sum((xs * gate_ref[...].astype(F32)).astype(BF16).astype(F32), axis=-1, keepdims=True)
        gte = jax.nn.sigmoid(gsum.astype(BF16).astype(F32))
        a = (xs * y_ref[pl.ds(r, SEG), :].astype(F32)).astype(BF16).astype(F32)
        out_ref[pl.ds(r, SEG), :] = (gte * a + (1.0 - gte) * b.astype(F32)).astype(BF16)

    def seg_body(s, mem):
        r = pl.multiple_of(s * SEG, SEG)
        xs = x_ref[pl.ds(r, SEG), :].astype(F32)
        h = jnp.concatenate([mem, xs], axis=0)
        qkvs = [None] * NH
        ps = [None] * NH
        os_ = [None] * NH

        def probs(hd):
            q = qkvs[hd][:, 0:DH].astype(BF16).astype(F32)
            k = qkvs[hd][:, DH:2 * DH].astype(BF16)
            sc = jnp.where(mask, _nt(q, k) * scale, -1e9)
            e = jnp.exp(sc - jnp.max(sc, axis=-1, keepdims=True))
            ps[hd] = (e / jnp.sum(e, axis=-1, keepdims=True)).astype(BF16).astype(F32)

        def values(hd):
            o = _nn(ps[hd], qkvs[hd][:, 2 * DH:3 * DH].astype(BF16))
            os_[hd] = o.astype(BF16).astype(F32)

        def slot(g):
            if g < NH:
                qkvs[g] = _nn(h, pltpu.bitcast(w2_ref[:, pl.ds(g * 3 * DH, 3 * DH)], BF16))
            if 0 <= g - L1 < NH:
                probs(g - L1)
            if 0 <= g - L2 < NH:
                values(g - L2)

        for g in range(NH):
            slot(g)
        acc = None
        nxt = NH
        for w in range(NH // WOG):
            while nxt < NH + L2 and (nxt - NH < (w + 1 - TOFF) * TRATE or nxt - L2 < (w + 1) * WOG):
                slot(nxt)
                nxt += 1
            og = jnp.concatenate(os_[w * WOG:(w + 1) * WOG], axis=1)
            wog = pltpu.bitcast(wo2_ref[pl.ds(w * WOG * DH // 2, WOG * DH // 2), :], BF16)
            part = _nn(og, wog)
            acc = part if acc is None else acc + part
        ob = acc.astype(BF16)
        epilogue(s, ob[MEM:])
        return ob[:MEM].astype(F32)

    def seg_pair(t, mem):
        @pl.when(t == XSPLIT // (SEG * SUNR))
        def _():
            x_copies[1].wait()

        for u in range(SUNR):
            mem = seg_body(t * SUNR + u, mem)
        out_copy(t).start()
        return mem

    jax.lax.fori_loop(0, NSEG // SUNR, seg_pair, mem0_ref[...].astype(F32))
    pltpu.make_async_copy(out_ref, o_hbm, sem_out).wait()


@functools.partial(jax.jit, static_argnames=("B_seg_len",))
def pallas_gated_mix__ssm_conv_h3__memory_aug_recurrent_mem_tr__prompt_kernel(
    A_q, A_k, A_v, A_shift_k, A_ssm_k, A_ssm_D, B_x, B_mem0, B_Wq, B_Wk, B_Wv, B_Wo, B_seg_len, gate_w,
):
    del B_x
    assert B_seg_len == SEG
    fwd, inv, sgn = _dft_consts()
    any_spec = pl.BlockSpec(memory_space=pl.ANY)
    vmem_spec = pl.BlockSpec(memory_space=pltpu.VMEM)
    out = pl.pallas_call(
        _kernel,
        out_shape=jax.ShapeDtypeStruct((S, D), BF16),
        in_specs=[any_spec] * 8 + [vmem_spec] * 7,
        out_specs=any_spec,
        scratch_shapes=[
            pltpu.VMEM((S, D), BF16),
            pltpu.VMEM((S, D), BF16),
            pltpu.VMEM((D // 2, 3 * NH * DH), U32),
            pltpu.VMEM((NH * DH // 2, D), U32),
            pltpu.VMEM((S, D), BF16),
            pltpu.SemaphoreType.DMA((3 * (D // CC) + 1,)),
            pltpu.SemaphoreType.DMA((6 * (CC // DCH) + D // CC,)),
            pltpu.SemaphoreType.DMA((2,)),
            pltpu.SemaphoreType.DMA(()),
        ],
        compiler_params=pltpu.CompilerParams(vmem_limit_bytes=120 * 1024 * 1024),
    )(
        A_q.reshape(S, D), A_k.reshape(S, D), A_v.reshape(S, D), A_ssm_k,
        B_Wq.reshape(D // 2, 2 * NH, DH), B_Wk.reshape(D // 2, 2 * NH, DH), B_Wv.reshape(D // 2, 2 * NH, DH),
        B_Wo.reshape(NH * DH, D),
        A_shift_k.T, A_ssm_D.reshape(1, D), gate_w.reshape(1, D), B_mem0.reshape(MEM, D),
        jnp.asarray(fwd.astype(jnp.bfloat16)), jnp.asarray(inv.astype(jnp.bfloat16)), jnp.asarray(sgn),
    )
    return out.reshape(1, S, D)
```

```python
import functools

import numpy as np
import jax
import jax.numpy as jnp
import jax.experimental.pallas as pl
import jax.experimental.pallas.tpu as pltpu

F32 = jnp.float32
BF16 = jnp.bfloat16
U32 = jnp.uint32

S = 2048
D = 1024
NH = 32
DH = 128
MEM = 8
SEG = 32
NSEG = S // SEG
L = MEM + SEG

TB = 256
NB = S // TB
CC = 256
DCH = 128
WPITCH = 24
XSPLIT = 128
UNR = 4
KPAD = 16
L1 = 2
L2 = 5
WOG = 4
TOFF = 1
TRATE = 1
SUNR = 2


def _dft_consts():
    n = 2 * TB
    t = np.arange(TB, dtype=np.float64)[None, :]
    f = (np.arange(TB, dtype=np.float64) + 0.5)[:, None]
    ang = 2.0 * np.pi * t * f / n
    fwd = np.concatenate([np.cos(ang), -np.sin(ang)], axis=0)
    inv = np.concatenate([np.cos(ang).T, -np.sin(ang).T], axis=1) * (2.0 / n)
    sgn = np.where(np.arange(8) % 2 == 0, 1.0, -1.0)[:, None] * np.ones((1, 128))
    return fwd.astype(np.float32), inv.astype(np.float32), sgn.astype(np.float32)


def _nt(a, b):
    return jax.lax.dot_general(a, b, (((1,), (1,)), ((), ())), preferred_element_type=F32)


def _nn(a, b):
    return jax.lax.dot_general(a, b, (((1,), (0,)), ((), ())), preferred_element_type=F32)


def unrolled(body):
    def run(j, c):
        for u in range(UNR):
            body(UNR * j + u, c)
        return c
    return run


def _kernel(xq_hbm, k_hbm, v_hbm, ssmk_hbm, wq_hbm, wk_hbm, wv_hbm, wo_hbm,
            shift_ref, ssmd_ref, gate_ref, mem0_ref, fwd_ref, inv_ref, sgn_ref,
            o_hbm,
            x_ref, y_ref, w2_ref, wo2_ref, out_ref, sem_in, sem_w, sem_x, sem_out):
    x_copies = [
        pltpu.make_async_copy(xq_hbm.at[pl.ds(0, XSPLIT), :], x_ref.at[pl.ds(0, XSPLIT), :], sem_x.at[0]),
        pltpu.make_async_copy(xq_hbm.at[pl.ds(XSPLIT, S - XSPLIT), :], x_ref.at[pl.ds(XSPLIT, S - XSPLIT), :],
                              sem_x.at[1]),
    ]

    def phase_a(k_ref, v_ref, ssmk_ref, kv_ref, uh_ref, kh_ref, raw_ref, stage_ref, stage_o_ref):
        n_cc = D // CC
        w_hbms = (wq_hbm, wk_hbm, wv_hbm)
        cpg = D // DCH // n_cc

        def filt_copy(cc):
            c0 = pl.multiple_of(cc * CC, CC)
            return pltpu.make_async_copy(ssmk_hbm.at[pl.ds(c0, CC), :], ssmk_ref.at[pl.ds(c0, CC), :],
                                         sem_in.at[3 * cc + 2])

        def in_copies(cc):
            c0 = pl.multiple_of(cc * CC, CC)
            return (
                pltpu.make_async_copy(k_hbm.at[:, pl.ds(c0, CC)], k_ref.at[pl.ds(KPAD, S), pl.ds(c0, CC)], sem_in.at[3 * cc]),
                pltpu.make_async_copy(v_hbm.at[:, pl.ds(c0, CC)], v_ref.at[:, pl.ds(c0, CC)], sem_in.at[3 * cc + 1]),
                filt_copy(cc),
            )

        def w_copies(cc, m, i):
            r0 = pl.multiple_of((cc * cpg + i) * (DCH // 2), DCH // 2)
            job = m * cpg + i
            return [pltpu.make_async_copy(w_hbms[m].at[pl.ds(r0, DCH // 2), :, :], raw_ref.at[job], sem_w.at[job])]

        wo_rows = NH * DH // n_cc

        def wo_copy(cc):
            r0 = pl.multiple_of(cc * wo_rows, wo_rows)
            return pltpu.make_async_copy(wo_hbm.at[pl.ds(r0, wo_rows), :], stage_o_ref.at[pl.ds(r0, wo_rows), :],
                                         sem_w.at[6 * cpg + cc])

        def wo_retile(cc):
            wo_copy(cc).wait()
            for b in range(wo_rows // 256):
                r0 = pl.multiple_of(cc * wo_rows + b * 256, 256)
                wo2_ref[pl.ds(pl.multiple_of(r0 // 2, 128), 128), :] = pltpu.bitcast(
                    stage_o_ref[pl.ds(r0, 256), :], U32)

        def retile(m, i, cc):
            jj = m * cpg + i
            c = cc * cpg + i
            for blk in range(DCH // 2 // 8):
                for par in range(2):
                    raw = raw_ref[jj, pl.ds(8 * blk, 8), pl.ds(par * NH, NH), :].reshape(8 * NH, DH)
                    stage_ref[m, par, pl.ds(8 * blk, 8), pl.ds(0, NH // 2), :] = (
                        pltpu.bitcast(raw, U32).reshape(8, NH // 2, DH))
            ev_ref = stage_ref.at[m, 0].reshape(DCH // 2 * WPITCH, DH)
            od_ref = stage_ref.at[m, 1].reshape(DCH // 2 * WPITCH, DH)
            for j in range(NH // 2):
                c0 = pl.multiple_of((2 * j * 3 + m) * DH, DH)
                c1 = pl.multiple_of(((2 * j + 1) * 3 + m) * DH, DH)
                for b in range(DCH // 16):
                    r0 = b * 8 * WPITCH + j
                    ev = ev_ref[pl.ds(r0, 8, stride=WPITCH), :]
                    od = od_ref[pl.ds(r0, 8, stride=WPITCH), :]
                    lo = (ev & jnp.uint32(0xFFFF)) | (od << 16)
                    hi = (ev >> 16) | (od & jnp.uint32(0xFFFF0000))
                    row = pl.multiple_of(c * (DCH // 2) + 8 * b, 8)
                    w2_ref[pl.ds(row, 8), pl.ds(c0, DH)] = lo
                    w2_ref[pl.ds(row, 8), pl.ds(c1, DH)] = hi

        filt_copy(0).start()
        k_ref[pl.ds(0, KPAD), :] = jnp.zeros((KPAD, D), BF16)

        def start_w(cc):
            for m in range(3):
                for i in range(cpg):
                    for c in w_copies(cc, m, i):
                        c.start()

        def chunk(cc, _):
            cur = in_copies(cc)
            cur[2].wait()

            @pl.when(cc == 0)
            def _():
                cur[0].start()
                cur[1].start()

            cs = pl.ds(pl.multiple_of(cc * CC, CC), CC)

            def filt_block(j, _):
                t0 = pl.multiple_of(j * TB, TB)
                kh_ref[j] = _nt(fwd_ref[...], ssmk_ref[cs, pl.ds(t0, TB)])
                return 0

            jax.lax.fori_loop(0, NB // UNR, unrolled(filt_block), 0)
            cur[0].wait()
            cur[1].wait()

            @pl.when(cc == 0)
            def _():
                start_w(cc)

            @pl.when(cc + 1 < n_cc)
            def _():
                for c in in_copies(cc + 1):
                    c.start()

            @pl.when(cc > 0)
            def _():
                wo_copy(cc - 1).start()

            @pl.when(cc == n_cc - 1)
            def _():
                wo_copy(cc).start()

            def fwd_block(j, _):
                t0 = pl.multiple_of(j * TB, TB)
                acc = None
                win = k_ref[pl.ds(t0, TB + KPAD), cs].astype(F32)
                for tap in range(4):
                    w = shift_ref[pl.ds(tap, 1), cs].astype(F32)
                    term = win[KPAD - tap:KPAD - tap + TB, :] * w
                    acc = term if acc is None else acc + term
                kvb = (acc * v_ref[pl.ds(t0, TB), cs].astype(F32)).astype(BF16)
                kv_ref[pl.ds(t0, TB), :] = kvb
                uh_ref[j] = _nn(fwd_ref[...], kvb)
                return 0

            jax.lax.fori_loop(0, NB // UNR, unrolled(fwd_block), 0)

            @pl.when(cc > 1)
            def _():
                wo_retile(cc - 2)

            @pl.when(cc == n_cc - 1)
            def _():
                x_copies[0].start()
                x_copies[1].start()

            sgn = sgn_ref[...]

            def spec_tile(ft, _):
                f0 = pl.multiple_of(ft * 8, 8)
                for lc in range(CC // 128):
                    ls = pl.ds(lc * 128, 128)
                    kr0 = [kh_ref[m, pl.ds(f0, 8), ls] for m in range(NB)]
                    ki0 = [kh_ref[m, pl.ds(TB + f0, 8), ls] for m in range(NB)]
                    kr = [kr0[0]] + [kr0[m] - sgn * ki0[m - 1] for m in range(1, NB)]
                    ki = [ki0[0]] + [ki0[m] + sgn * kr0[m - 1] for m in range(1, NB)]
                    ur = [uh_ref[j, pl.ds(f0, 8), ls] for j in range(NB)]
                    ui = [uh_ref[j, pl.ds(TB + f0, 8), ls] for j in range(NB)]
                    for i in range(NB):
                        zr = None
                        zi = None
                        for m in range(i + 1):
                            tr = kr[m] * ur[i - m] - ki[m] * ui[i - m]
                            ti = kr[m] * ui[i - m] + ki[m] * ur[i - m]
                            zr = tr if zr is None else zr + tr
                            zi = ti if zi is None else zi + ti
                        kh_ref[i, pl.ds(f0, 8), ls] = zr
                        kh_ref[i, pl.ds(TB + f0, 8), ls] = zi
                return 0

            jax.lax.fori_loop(0, TB // 8, spec_tile, 0)

            def inv_block(i, _):
                t0 = pl.multiple_of(i * TB, TB)
                yb = _nn(inv_ref[...], kh_ref[i].astype(BF16))
                yb = yb + kv_ref[pl.ds(t0, TB), :].astype(F32) * ssmd_ref[:, cs].astype(F32)
                y_ref[pl.ds(t0, TB), cs] = yb.astype(BF16)
                return 0

            def inv_retile(i, c):
                for m in range(3):
                    for cp in w_copies(cc, m, i):
                        cp.wait()
                unrolled(inv_block)(i, c)
                for m in range(3):
                    retile(m, i, cc)

                @pl.when(cc + 1 < n_cc)
                def _():
                    for m in range(3):
                        for cp in w_copies(cc + 1, m, i):
                            cp.start()

                return c

            assert NB // UNR == cpg
            jax.lax.fori_loop(0, cpg, inv_retile, 0)
            return 0

        jax.lax.fori_loop(0, n_cc, chunk, 0)

        wo_retile(n_cc - 2)
        wo_retile(n_cc - 1)
        x_copies[0].wait()

    pl.run_scoped(
        phase_a,
        pltpu.VMEM((KPAD + S, D), BF16), pltpu.VMEM((S, D), BF16), pltpu.VMEM((D, S), BF16),
        pltpu.VMEM((S, CC), BF16),
        pltpu.VMEM((NB, 2 * TB, CC), F32), pltpu.VMEM((NB, 2 * TB, CC), F32),
        pltpu.VMEM((3 * (CC // DCH), DCH // 2, 2 * NH, DH), BF16), pltpu.VMEM((3, 2, DCH // 2, WPITCH, DH), U32), pltpu.VMEM((NH * DH, D), BF16),
    )

    scale = DH ** -0.5
    row = jax.lax.broadcasted_iota(jnp.int32, (L, L), 0)
    col = jax.lax.broadcasted_iota(jnp.int32, (L, L), 1)
    mask = (row < MEM) | (row >= col)

    def out_copy(t):
        r = pl.multiple_of(t * (SEG * SUNR), SEG * SUNR)
        return pltpu.make_async_copy(out_ref.at[pl.ds(r, SEG * SUNR), :], o_hbm.at[pl.ds(r, SEG * SUNR), :], sem_out)

    def epilogue(s, b):
        r = pl.multiple_of(s * SEG, SEG)
        xs = x_ref[pl.ds(r, SEG), :].astype(F32)
        gsum = jnp.sum((xs * gate_ref[...].astype(F32)).astype(BF16).astype(F32), axis=-1, keepdims=True)
        gte = jax.nn.sigmoid(gsum.astype(BF16).astype(F32))
        a = (xs * y_ref[pl.ds(r, SEG), :].astype(F32)).astype(BF16).astype(F32)
        out_ref[pl.ds(r, SEG), :] = (gte * a + (1.0 - gte) * b.astype(F32)).astype(BF16)

    def seg_body(s, mem):
        r = pl.multiple_of(s * SEG, SEG)
        xs = x_ref[pl.ds(r, SEG), :].astype(F32)
        h = jnp.concatenate([mem, xs], axis=0)
        qkvs = [None] * NH
        ps = [None] * NH
        os_ = [None] * NH

        def probs(hd):
            q = qkvs[hd][:, 0:DH].astype(BF16).astype(F32)
            k = qkvs[hd][:, DH:2 * DH].astype(BF16)
            sc = jnp.where(mask, _nt(q, k) * scale, -1e9)
            e = jnp.exp(sc - jnp.max(sc, axis=-1, keepdims=True))
            ps[hd] = (e / jnp.sum(e, axis=-1, keepdims=True)).astype(BF16).astype(F32)

        def values(hd):
            o = _nn(ps[hd], qkvs[hd][:, 2 * DH:3 * DH].astype(BF16))
            os_[hd] = o.astype(BF16).astype(F32)

        def slot(g):
            if g < NH:
                qkvs[g] = _nn(h, pltpu.bitcast(w2_ref[:, pl.ds(g * 3 * DH, 3 * DH)], BF16))
            if 0 <= g - L1 < NH:
                probs(g - L1)
            if 0 <= g - L2 < NH:
                values(g - L2)

        for g in range(NH):
            slot(g)
        acc = None
        nxt = NH
        for w in range(NH // WOG):
            while nxt < NH + L2 and (nxt - NH < (w + 1 - TOFF) * TRATE or nxt - L2 < (w + 1) * WOG):
                slot(nxt)
                nxt += 1
            og = jnp.concatenate(os_[w * WOG:(w + 1) * WOG], axis=1)
            wog = pltpu.bitcast(wo2_ref[pl.ds(w * WOG * DH // 2, WOG * DH // 2), :], BF16)
            part = _nn(og, wog)
            acc = part if acc is None else acc + part
        ob = acc.astype(BF16)
        epilogue(s, ob[MEM:])
        return ob[:MEM].astype(F32)

    def seg_pair(t, mem):
        @pl.when(t == XSPLIT // (SEG * SUNR))
        def _():
            x_copies[1].wait()

        for u in range(SUNR):
            mem = seg_body(t * SUNR + u, mem)
        out_copy(t).start()
        return mem

    jax.lax.fori_loop(0, NSEG // SUNR, seg_pair, mem0_ref[...].astype(F32))
    pltpu.make_async_copy(out_ref, o_hbm, sem_out).wait()


@functools.partial(jax.jit, static_argnames=("B_seg_len",))
def pallas_gated_mix__ssm_conv_h3__memory_aug_recurrent_mem_tr__prompt_kernel(
    A_q, A_k, A_v, A_shift_k, A_ssm_k, A_ssm_D, B_x, B_mem0, B_Wq, B_Wk, B_Wv, B_Wo, B_seg_len, gate_w,
):
    del B_x
    assert B_seg_len == SEG
    fwd, inv, sgn = _dft_consts()
    any_spec = pl.BlockSpec(memory_space=pl.ANY)
    vmem_spec = pl.BlockSpec(memory_space=pltpu.VMEM)
    out = pl.pallas_call(
        _kernel,
        out_shape=jax.ShapeDtypeStruct((S, D), BF16),
        in_specs=[any_spec] * 8 + [vmem_spec] * 7,
        out_specs=any_spec,
        scratch_shapes=[
            pltpu.VMEM((S, D), BF16),
            pltpu.VMEM((S, D), BF16),
            pltpu.VMEM((D // 2, 3 * NH * DH), U32),
            pltpu.VMEM((NH * DH // 2, D), U32),
            pltpu.VMEM((S, D), BF16),
            pltpu.SemaphoreType.DMA((3 * (D // CC) + 1,)),
            pltpu.SemaphoreType.DMA((6 * (CC // DCH) + D // CC,)),
            pltpu.SemaphoreType.DMA((2,)),
            pltpu.SemaphoreType.DMA(()),
        ],
        compiler_params=pltpu.CompilerParams(vmem_limit_bytes=120 * 1024 * 1024),
    )(
        A_q.reshape(S, D), A_k.reshape(S, D), A_v.reshape(S, D), A_ssm_k,
        B_Wq.reshape(D // 2, 2 * NH, DH), B_Wk.reshape(D // 2, 2 * NH, DH), B_Wv.reshape(D // 2, 2 * NH, DH),
        B_Wo.reshape(NH * DH, D),
        A_shift_k.T, A_ssm_D.reshape(1, D), gate_w.reshape(1, D), B_mem0.reshape(MEM, D),
        jnp.asarray(fwd.astype(jnp.bfloat16)), jnp.asarray(inv.astype(jnp.bfloat16)), jnp.asarray(sgn),
    )
    return out.reshape(1, S, D)
```

```python
import functools

import numpy as np
import jax
import jax.numpy as jnp
import jax.experimental.pallas as pl
import jax.experimental.pallas.tpu as pltpu

F32 = jnp.float32
BF16 = jnp.bfloat16
U32 = jnp.uint32

S = 2048
D = 1024
NH = 32
DH = 128
MEM = 8
SEG = 32
NSEG = S // SEG
L = MEM + SEG

TB = 256
NB = S // TB
CC = 256
DCH = 128
WPITCH = 24
XSPLIT = 128
UNR = 4
KPAD = 16
L1 = 2
L2 = 5
WOG = 4
TOFF = 1
SUNR = 2


def _dft_consts():
    n = 2 * TB
    t = np.arange(TB, dtype=np.float64)[None, :]
    f = (np.arange(TB, dtype=np.float64) + 0.5)[:, None]
    ang = 2.0 * np.pi * t * f / n
    fwd = np.concatenate([np.cos(ang), -np.sin(ang)], axis=0)
    inv = np.concatenate([np.cos(ang).T, -np.sin(ang).T], axis=1) * (2.0 / n)
    sgn = np.where(np.arange(8) % 2 == 0, 1.0, -1.0)[:, None] * np.ones((1, 128))
    return fwd.astype(np.float32), inv.astype(np.float32), sgn.astype(np.float32)


def _nt(a, b):
    return jax.lax.dot_general(a, b, (((1,), (1,)), ((), ())), preferred_element_type=F32)


def _nn(a, b):
    return jax.lax.dot_general(a, b, (((1,), (0,)), ((), ())), preferred_element_type=F32)


def unrolled(body):
    def run(j, c):
        for u in range(UNR):
            body(UNR * j + u, c)
        return c
    return run


def _kernel(xq_hbm, k_hbm, v_hbm, ssmk_hbm, wq_hbm, wk_hbm, wv_hbm, wo_hbm,
            shift_ref, ssmd_ref, gate_ref, mem0_ref, fwd_ref, inv_ref, sgn_ref,
            o_hbm,
            x_ref, y_ref, w2_ref, wo2_ref, out_ref, sem_in, sem_w, sem_x, sem_out):
    x_copies = [
        pltpu.make_async_copy(xq_hbm.at[pl.ds(0, XSPLIT), :], x_ref.at[pl.ds(0, XSPLIT), :], sem_x.at[0]),
        pltpu.make_async_copy(xq_hbm.at[pl.ds(XSPLIT, S - XSPLIT), :], x_ref.at[pl.ds(XSPLIT, S - XSPLIT), :],
                              sem_x.at[1]),
    ]

    def phase_a(k_ref, v_ref, ssmk_ref, kv_ref, uh_ref, kh_ref, raw_ref, stage_ref, stage_o_ref):
        n_cc = D // CC
        w_hbms = (wq_hbm, wk_hbm, wv_hbm)
        cpg = D // DCH // n_cc

        def filt_copy(cc):
            c0 = pl.multiple_of(cc * CC, CC)
            return pltpu.make_async_copy(ssmk_hbm.at[pl.ds(c0, CC), :], ssmk_ref.at[pl.ds(c0, CC), :],
                                         sem_in.at[3 * cc + 2])

        def in_copies(cc):
            c0 = pl.multiple_of(cc * CC, CC)
            return (
                pltpu.make_async_copy(k_hbm.at[:, pl.ds(c0, CC)], k_ref.at[pl.ds(KPAD, S), pl.ds(c0, CC)], sem_in.at[3 * cc]),
                pltpu.make_async_copy(v_hbm.at[:, pl.ds(c0, CC)], v_ref.at[:, pl.ds(c0, CC)], sem_in.at[3 * cc + 1]),
                filt_copy(cc),
            )

        def w_copies(cc, m, i):
            r0 = pl.multiple_of((cc * cpg + i) * (DCH // 2), DCH // 2)
            job = m * cpg + i
            return [pltpu.make_async_copy(w_hbms[m].at[pl.ds(r0, DCH // 2), :, :], raw_ref.at[job], sem_w.at[job])]

        wo_rows = NH * DH // n_cc

        def wo_copy(cc):
            r0 = pl.multiple_of(cc * wo_rows, wo_rows)
            return pltpu.make_async_copy(wo_hbm.at[pl.ds(r0, wo_rows), :], stage_o_ref.at[pl.ds(r0, wo_rows), :],
                                         sem_w.at[3 * cpg + cc])

        def wo_retile(cc):
            wo_copy(cc).wait()
            for b in range(wo_rows // 256):
                r0 = pl.multiple_of(cc * wo_rows + b * 256, 256)
                wo2_ref[pl.ds(pl.multiple_of(r0 // 2, 128), 128), :] = pltpu.bitcast(
                    stage_o_ref[pl.ds(r0, 256), :], U32)

        def retile(m, i, cc):
            jj = m * cpg + i
            c = cc * cpg + i
            for blk in range(DCH // 2 // 8):
                for par in range(2):
                    raw = raw_ref[jj, pl.ds(8 * blk, 8), pl.ds(par * NH, NH), :].reshape(8 * NH, DH)
                    words = pltpu.bitcast(raw, U32)
                    for r in range(8):
                        stage_ref[m, par, pl.ds((8 * blk + r) * WPITCH, NH // 2), :] = (
                            words[r * (NH // 2):(r + 1) * (NH // 2)])
            for j in range(NH // 2):
                c0 = (2 * j * 3 + m) * DH
                c1 = ((2 * j + 1) * 3 + m) * DH
                for b in range(DCH // 16):
                    r0 = b * 8 * WPITCH + j
                    ev = stage_ref[m, 0, pl.ds(r0, 8, stride=WPITCH), :]
                    od = stage_ref[m, 1, pl.ds(r0, 8, stride=WPITCH), :]
                    lo = (ev & jnp.uint32(0xFFFF)) | (od << 16)
                    hi = (ev >> 16) | (od & jnp.uint32(0xFFFF0000))
                    row = pl.multiple_of(c * (DCH // 2) + 8 * b, 8)
                    w2_ref[pl.ds(row, 8), pl.ds(c0, DH)] = lo
                    w2_ref[pl.ds(row, 8), pl.ds(c1, DH)] = hi

        filt_copy(0).start()
        k_ref[pl.ds(0, KPAD), :] = jnp.zeros((KPAD, D), BF16)

        def start_w(cc):
            for m in range(3):
                for i in range(cpg):
                    for c in w_copies(cc, m, i):
                        c.start()

        def chunk(cc, _):
            cur = in_copies(cc)
            cur[2].wait()

            @pl.when(cc == 0)
            def _():
                cur[0].start()
                cur[1].start()

            cs = pl.ds(pl.multiple_of(cc * CC, CC), CC)

            def filt_block(j, _):
                t0 = pl.multiple_of(j * TB, TB)
                kh_ref[j] = _nt(fwd_ref[...], ssmk_ref[cs, pl.ds(t0, TB)])
                return 0

            jax.lax.fori_loop(0, NB // UNR, unrolled(filt_block), 0)
            cur[0].wait()
            cur[1].wait()

            @pl.when(cc == 0)
            def _():
                start_w(cc)

            @pl.when(cc + 1 < n_cc)
            def _():
                for c in in_copies(cc + 1):
                    c.start()

            @pl.when(cc > 0)
            def _():
                wo_copy(cc - 1).start()

            @pl.when(cc == n_cc - 1)
            def _():
                wo_copy(cc).start()

            def fwd_block(j, _):
                t0 = pl.multiple_of(j * TB, TB)
                acc = None
                win = k_ref[pl.ds(t0, TB + KPAD), cs].astype(F32)
                for tap in range(4):
                    w = shift_ref[pl.ds(tap, 1), cs].astype(F32)
                    term = win[KPAD - tap:KPAD - tap + TB, :] * w
                    acc = term if acc is None else acc + term
                kvb = (acc * v_ref[pl.ds(t0, TB), cs].astype(F32)).astype(BF16)
                kv_ref[pl.ds(t0, TB), :] = kvb
                uh_ref[j] = _nn(fwd_ref[...], kvb)
                return 0

            jax.lax.fori_loop(0, NB // UNR, unrolled(fwd_block), 0)

            @pl.when(cc > 1)
            def _():
                wo_retile(cc - 2)

            @pl.when(cc == n_cc - 1)
            def _():
                x_copies[0].start()
                x_copies[1].start()

            sgn = sgn_ref[...]

            def spec_tile(ft, _):
                f0 = pl.multiple_of(ft * 8, 8)
                for lc in range(CC // 128):
                    ls = pl.ds(lc * 128, 128)
                    kr0 = [kh_ref[m, pl.ds(f0, 8), ls] for m in range(NB)]
                    ki0 = [kh_ref[m, pl.ds(TB + f0, 8), ls] for m in range(NB)]
                    kr = [kr0[0]] + [kr0[m] - sgn * ki0[m - 1] for m in range(1, NB)]
                    ki = [ki0[0]] + [ki0[m] + sgn * kr0[m - 1] for m in range(1, NB)]
                    ur = [uh_ref[j, pl.ds(f0, 8), ls] for j in range(NB)]
                    ui = [uh_ref[j, pl.ds(TB + f0, 8), ls] for j in range(NB)]
                    for i in range(NB):
                        zr = None
                        zi = None
                        for m in range(i + 1):
                            tr = kr[m] * ur[i - m] - ki[m] * ui[i - m]
                            ti = kr[m] * ui[i - m] + ki[m] * ur[i - m]
                            zr = tr if zr is None else zr + tr
                            zi = ti if zi is None else zi + ti
                        kh_ref[i, pl.ds(f0, 8), ls] = zr
                        kh_ref[i, pl.ds(TB + f0, 8), ls] = zi
                return 0

            jax.lax.fori_loop(0, TB // 8, spec_tile, 0)

            def inv_block(i, _):
                t0 = pl.multiple_of(i * TB, TB)
                yb = _nn(inv_ref[...], kh_ref[i].astype(BF16))
                yb = yb + kv_ref[pl.ds(t0, TB), :].astype(F32) * ssmd_ref[:, cs].astype(F32)
                y_ref[pl.ds(t0, TB), cs] = yb.astype(BF16)
                return 0

            def inv_retile(i, c):
                for m in range(3):
                    for cp in w_copies(cc, m, i):
                        cp.wait()
                unrolled(inv_block)(i, c)
                for m in range(3):
                    retile(m, i, cc)

                @pl.when(cc + 1 < n_cc)
                def _():
                    for m in range(3):
                        for cp in w_copies(cc + 1, m, i):
                            cp.start()

                return c

            assert NB // UNR == cpg
            jax.lax.fori_loop(0, cpg, inv_retile, 0)
            return 0

        jax.lax.fori_loop(0, n_cc, chunk, 0)

        wo_retile(n_cc - 2)
        wo_retile(n_cc - 1)
        x_copies[0].wait()

    pl.run_scoped(
        phase_a,
        pltpu.VMEM((KPAD + S, D), BF16), pltpu.VMEM((S, D), BF16), pltpu.VMEM((D, S), BF16),
        pltpu.VMEM((S, CC), BF16),
        pltpu.VMEM((NB, 2 * TB, CC), F32), pltpu.VMEM((NB, 2 * TB, CC), F32),
        pltpu.VMEM((3 * (CC // DCH), DCH // 2, 2 * NH, DH), BF16), pltpu.VMEM((3, 2, DCH // 2 * WPITCH, DH), U32), pltpu.VMEM((NH * DH, D), BF16),
    )

    scale = DH ** -0.5
    row = jax.lax.broadcasted_iota(jnp.int32, (L, L), 0)
    col = jax.lax.broadcasted_iota(jnp.int32, (L, L), 1)
    mask = (row < MEM) | (row >= col)

    def out_copy(t):
        r = pl.multiple_of(t * (SEG * SUNR), SEG * SUNR)
        return pltpu.make_async_copy(out_ref.at[pl.ds(r, SEG * SUNR), :], o_hbm.at[pl.ds(r, SEG * SUNR), :], sem_out)

    def epilogue(s, b):
        r = pl.multiple_of(s * SEG, SEG)
        xs = x_ref[pl.ds(r, SEG), :].astype(F32)
        gsum = jnp.sum((xs * gate_ref[...].astype(F32)).astype(BF16).astype(F32), axis=-1, keepdims=True)
        gte = jax.nn.sigmoid(gsum.astype(BF16).astype(F32))
        a = (xs * y_ref[pl.ds(r, SEG), :].astype(F32)).astype(BF16).astype(F32)
        out_ref[pl.ds(r, SEG), :] = (gte * a + (1.0 - gte) * b.astype(F32)).astype(BF16)

    def seg_body(s, mem):
        r = pl.multiple_of(s * SEG, SEG)
        xs = x_ref[pl.ds(r, SEG), :].astype(F32)
        h = jnp.concatenate([mem, xs], axis=0)
        qkvs = [None] * NH
        ps = [None] * NH
        os_ = [None] * NH

        def probs(hd):
            q = qkvs[hd][:, 0:DH].astype(BF16).astype(F32)
            k = qkvs[hd][:, DH:2 * DH].astype(BF16)
            sc = jnp.where(mask, _nt(q, k) * scale, -1e9)
            e = jnp.exp(sc - jnp.max(sc, axis=-1, keepdims=True))
            ps[hd] = (e / jnp.sum(e, axis=-1, keepdims=True)).astype(BF16).astype(F32)

        def values(hd):
            o = _nn(ps[hd], qkvs[hd][:, 2 * DH:3 * DH].astype(BF16))
            os_[hd] = o.astype(BF16).astype(F32)

        def slot(g):
            if g < NH:
                qkvs[g] = _nn(h, pltpu.bitcast(w2_ref[:, pl.ds(g * 3 * DH, 3 * DH)], BF16))
            if 0 <= g - L1 < NH:
                probs(g - L1)
            if 0 <= g - L2 < NH:
                values(g - L2)

        for g in range(NH):
            slot(g)
        acc = None
        nxt = NH
        for w in range(NH // WOG):
            while nxt < NH + L2 and (nxt - NH < w + 1 - TOFF or nxt - L2 < (w + 1) * WOG):
                slot(nxt)
                nxt += 1
            og = jnp.concatenate(os_[w * WOG:(w + 1) * WOG], axis=1)
            wog = pltpu.bitcast(wo2_ref[pl.ds(w * WOG * DH // 2, WOG * DH // 2), :], BF16)
            part = _nn(og, wog)
            acc = part if acc is None else acc + part
        ob = acc.astype(BF16)
        epilogue(s, ob[MEM:])
        return ob[:MEM].astype(F32)

    def seg_pair(t, mem):
        @pl.when(t == XSPLIT // (SEG * SUNR))
        def _():
            x_copies[1].wait()

        for u in range(SUNR):
            mem = seg_body(t * SUNR + u, mem)
        out_copy(t).start()
        return mem

    jax.lax.fori_loop(0, NSEG // SUNR, seg_pair, mem0_ref[...].astype(F32))
    pltpu.make_async_copy(out_ref, o_hbm, sem_out).wait()


@functools.partial(jax.jit, static_argnames=("B_seg_len",))
def pallas_gated_mix__ssm_conv_h3__memory_aug_recurrent_mem_tr__prompt_kernel(
    A_q, A_k, A_v, A_shift_k, A_ssm_k, A_ssm_D, B_x, B_mem0, B_Wq, B_Wk, B_Wv, B_Wo, B_seg_len, gate_w,
):
    del B_x
    assert B_seg_len == SEG
    fwd, inv, sgn = _dft_consts()
    any_spec = pl.BlockSpec(memory_space=pl.ANY)
    vmem_spec = pl.BlockSpec(memory_space=pltpu.VMEM)
    out = pl.pallas_call(
        _kernel,
        out_shape=jax.ShapeDtypeStruct((S, D), BF16),
        in_specs=[any_spec] * 8 + [vmem_spec] * 7,
        out_specs=any_spec,
        scratch_shapes=[
            pltpu.VMEM((S, D), BF16),
            pltpu.VMEM((S, D), BF16),
            pltpu.VMEM((D // 2, 3 * NH * DH), U32),
            pltpu.VMEM((NH * DH // 2, D), U32),
            pltpu.VMEM((S, D), BF16),
            pltpu.SemaphoreType.DMA((3 * (D // CC) + 1,)),
            pltpu.SemaphoreType.DMA((3 * (CC // DCH) + D // CC,)),
            pltpu.SemaphoreType.DMA((2,)),
            pltpu.SemaphoreType.DMA(()),
        ],
        compiler_params=pltpu.CompilerParams(vmem_limit_bytes=120 * 1024 * 1024),
    )(
        A_q.reshape(S, D), A_k.reshape(S, D), A_v.reshape(S, D), A_ssm_k,
        B_Wq.reshape(D // 2, 2 * NH, DH), B_Wk.reshape(D // 2, 2 * NH, DH), B_Wv.reshape(D // 2, 2 * NH, DH),
        B_Wo.reshape(NH * DH, D),
        A_shift_k.T, A_ssm_D.reshape(1, D), gate_w.reshape(1, D), B_mem0.reshape(MEM, D),
        jnp.asarray(fwd.astype(jnp.bfloat16)), jnp.asarray(inv.astype(jnp.bfloat16)), jnp.asarray(sgn),
    )
    return out.reshape(1, S, D)
```

```python
import functools

import numpy as np
import jax
import jax.numpy as jnp
import jax.experimental.pallas as pl
import jax.experimental.pallas.tpu as pltpu

F32 = jnp.float32
BF16 = jnp.bfloat16
U32 = jnp.uint32

S = 2048
D = 1024
NH = 32
DH = 128
MEM = 8
SEG = 32
NSEG = S // SEG
L = MEM + SEG

TB = 256
NB = S // TB
CC = 256
DCH = 128
WPITCH = 24
XSPLIT = 128
UNR = 4
KPAD = 16
L1 = 2
L2 = 5
WOG = 4
TOFF = 1
SUNR = 2


def _dft_consts():
    n = 2 * TB
    t = np.arange(TB, dtype=np.float64)[None, :]
    f = (np.arange(TB, dtype=np.float64) + 0.5)[:, None]
    ang = 2.0 * np.pi * t * f / n
    fwd = np.concatenate([np.cos(ang), -np.sin(ang)], axis=0)
    inv = np.concatenate([np.cos(ang).T, -np.sin(ang).T], axis=1) * (2.0 / n)
    sgn = np.where(np.arange(8) % 2 == 0, 1.0, -1.0)[:, None] * np.ones((1, 128))
    return fwd.astype(np.float32), inv.astype(np.float32), sgn.astype(np.float32)


def _nt(a, b):
    return jax.lax.dot_general(a, b, (((1,), (1,)), ((), ())), preferred_element_type=F32)


def _nn(a, b):
    return jax.lax.dot_general(a, b, (((1,), (0,)), ((), ())), preferred_element_type=F32)


def unrolled(body):
    def run(j, c):
        for u in range(UNR):
            body(UNR * j + u, c)
        return c
    return run


def _kernel(xq_hbm, k_hbm, v_hbm, ssmk_hbm, wq_hbm, wk_hbm, wv_hbm, wo_hbm,
            shift_ref, ssmd1_ref, gate1_ref, mem0_ref, fwd_ref, inv_ref, sgn_ref,
            o_hbm,
            x_ref, y_ref, w2_ref, wo2_ref, out_ref, ssmd_ref, gate_ref, sem_in, sem_w, sem_x, sem_out):
    x_copies = [
        pltpu.make_async_copy(xq_hbm.at[pl.ds(0, XSPLIT), :], x_ref.at[pl.ds(0, XSPLIT), :], sem_x.at[0]),
        pltpu.make_async_copy(xq_hbm.at[pl.ds(XSPLIT, S - XSPLIT), :], x_ref.at[pl.ds(XSPLIT, S - XSPLIT), :],
                              sem_x.at[1]),
    ]

    ssmd_ref[...] = ssmd1_ref[...].astype(F32).reshape(1, D)
    gate_ref[...] = gate1_ref[...].astype(F32).reshape(1, D)

    def phase_a(k_ref, v_ref, ssmk_ref, kv_ref, uh_ref, kh0_ref, kh1_ref, raw_ref, stage_ref, stage_o_ref):
        n_cc = D // CC
        kh_refs = (kh0_ref, kh1_ref)
        w_hbms = (wq_hbm, wk_hbm, wv_hbm)
        cpg = D // DCH // n_cc

        def filt_copy(cc):
            c0 = pl.multiple_of(cc * CC, CC)
            return pltpu.make_async_copy(ssmk_hbm.at[pl.ds(c0, CC), :], ssmk_ref.at[pl.ds(c0, CC), :],
                                         sem_in.at[3 * cc + 2])

        def in_copies(cc):
            c0 = pl.multiple_of(cc * CC, CC)
            return (
                pltpu.make_async_copy(k_hbm.at[:, pl.ds(c0, CC)], k_ref.at[pl.ds(KPAD, S), pl.ds(c0, CC)], sem_in.at[3 * cc]),
                pltpu.make_async_copy(v_hbm.at[:, pl.ds(c0, CC)], v_ref.at[:, pl.ds(c0, CC)], sem_in.at[3 * cc + 1]),
            )

        def w_copies(cc, m, i):
            r0 = pl.multiple_of((cc * cpg + i) * (DCH // 2), DCH // 2)
            job = m * cpg + i
            return [pltpu.make_async_copy(w_hbms[m].at[pl.ds(r0, DCH // 2), :, :], raw_ref.at[job], sem_w.at[job])]

        wo_rows = NH * DH // n_cc

        def wo_copy(cc):
            r0 = pl.multiple_of(cc * wo_rows, wo_rows)
            return pltpu.make_async_copy(wo_hbm.at[pl.ds(r0, wo_rows), :], stage_o_ref.at[pl.ds(r0, wo_rows), :],
                                         sem_w.at[3 * cpg + cc])

        def wo_retile(cc):
            wo_copy(cc).wait()
            for b in range(wo_rows // 256):
                r0 = pl.multiple_of(cc * wo_rows + b * 256, 256)
                wo2_ref[pl.ds(pl.multiple_of(r0 // 2, 128), 128), :] = pltpu.bitcast(
                    stage_o_ref[pl.ds(r0, 256), :], U32)

        def retile(m, i, cc):
            jj = m * cpg + i
            c = cc * cpg + i
            for blk in range(DCH // 2 // 8):
                for par in range(2):
                    raw = raw_ref[jj, pl.ds(8 * blk, 8), pl.ds(par * NH, NH), :].reshape(8 * NH, DH)
                    words = pltpu.bitcast(raw, U32)
                    for r in range(8):
                        stage_ref[m, par, pl.ds((8 * blk + r) * WPITCH, NH // 2), :] = (
                            words[r * (NH // 2):(r + 1) * (NH // 2)])
            for j in range(NH // 2):
                c0 = (2 * j * 3 + m) * DH
                c1 = ((2 * j + 1) * 3 + m) * DH
                for b in range(DCH // 16):
                    r0 = b * 8 * WPITCH + j
                    ev = stage_ref[m, 0, pl.ds(r0, 8, stride=WPITCH), :]
                    od = stage_ref[m, 1, pl.ds(r0, 8, stride=WPITCH), :]
                    lo = (ev & jnp.uint32(0xFFFF)) | (od << 16)
                    hi = (ev >> 16) | (od & jnp.uint32(0xFFFF0000))
                    row = pl.multiple_of(c * (DCH // 2) + 8 * b, 8)
                    w2_ref[pl.ds(row, 8), pl.ds(c0, DH)] = lo
                    w2_ref[pl.ds(row, 8), pl.ds(c1, DH)] = hi

        def filt_block(j, cc, slot):
            t0 = pl.multiple_of(j * TB, TB)
            cs = pl.ds(pl.multiple_of(cc * CC, CC), CC)
            kh_refs[slot][j] = _nt(fwd_ref[...], ssmk_ref[cs, pl.ds(t0, TB)])

        filt_copy(0).start()
        k_ref[pl.ds(0, KPAD), :] = jnp.zeros((KPAD, D), BF16)
        filt_copy(0).wait()
        for c in in_copies(0):
            c.start()
        filt_copy(1).start()
        jax.lax.fori_loop(0, NB // UNR, unrolled(lambda j, c: filt_block(j, 0, 0)), 0)

        def start_w(cc):
            for m in range(3):
                for i in range(cpg):
                    for c in w_copies(cc, m, i):
                        c.start()

        def chunk(cc, _):
            par = cc % 2
            for c in in_copies(cc):
                c.wait()

            @pl.when(cc == 0)
            def _():
                start_w(cc)

            @pl.when(cc + 1 < n_cc)
            def _():
                for c in in_copies(cc + 1):
                    c.start()

            @pl.when(cc > 0)
            def _():
                wo_copy(cc - 1).start()

            @pl.when(cc == n_cc - 1)
            def _():
                wo_copy(cc).start()

            cs = pl.ds(pl.multiple_of(cc * CC, CC), CC)

            def fwd_block(j, _):
                t0 = pl.multiple_of(j * TB, TB)
                acc = None
                win = k_ref[pl.ds(t0, TB + KPAD), cs].astype(F32)
                for tap in range(4):
                    w = shift_ref[pl.ds(tap, 1), cs].astype(F32)
                    term = win[KPAD - tap:KPAD - tap + TB, :] * w
                    acc = term if acc is None else acc + term
                kvb = (acc * v_ref[pl.ds(t0, TB), cs].astype(F32)).astype(BF16)
                kv_ref[pl.ds(t0, TB), :] = kvb
                uh_ref[j] = _nn(fwd_ref[...], kvb)
                return 0

            jax.lax.fori_loop(0, NB // UNR, unrolled(fwd_block), 0)

            @pl.when(cc > 1)
            def _():
                wo_retile(cc - 2)

            @pl.when(cc == n_cc - 1)
            def _():
                x_copies[0].start()
                x_copies[1].start()

            sgn = sgn_ref[...]

            def spec_tile(ft, _):
                f0 = pl.multiple_of(ft * 8, 8)
                for lc in range(CC // 128):
                    ls = pl.ds(lc * 128, 128)
                    kr0 = [kh_refs[par][m, pl.ds(f0, 8), ls] for m in range(NB)]
                    ki0 = [kh_refs[par][m, pl.ds(TB + f0, 8), ls] for m in range(NB)]
                    kr = [kr0[0]] + [kr0[m] - sgn * ki0[m - 1] for m in range(1, NB)]
                    ki = [ki0[0]] + [ki0[m] + sgn * kr0[m - 1] for m in range(1, NB)]
                    ur = [uh_ref[j, pl.ds(f0, 8), ls] for j in range(NB)]
                    ui = [uh_ref[j, pl.ds(TB + f0, 8), ls] for j in range(NB)]
                    for i in range(NB):
                        zr = None
                        zi = None
                        for m in range(i + 1):
                            tr = kr[m] * ur[i - m] - ki[m] * ui[i - m]
                            ti = kr[m] * ui[i - m] + ki[m] * ur[i - m]
                            zr = tr if zr is None else zr + tr
                            zi = ti if zi is None else zi + ti
                        kh_refs[par][i, pl.ds(f0, 8), ls] = zr
                        kh_refs[par][i, pl.ds(TB + f0, 8), ls] = zi
                return 0

            @pl.when(cc + 2 < n_cc)
            def _():
                filt_copy(cc + 2).start()

            @pl.when(cc + 1 < n_cc)
            def _():
                filt_copy(cc + 1).wait()

            tpb = TB // 8 // NB

            def spec_filt(j, c):
                if cc + 1 < n_cc:
                    filt_block(j, cc + 1, 1 - par)
                for u in range(tpb):
                    spec_tile(j * tpb + u, c)
                return c

            jax.lax.fori_loop(0, NB, spec_filt, 0)

            def inv_block(i, _):
                t0 = pl.multiple_of(i * TB, TB)
                yb = _nn(inv_ref[...], kh_refs[par][i].astype(BF16))
                yb = yb + kv_ref[pl.ds(t0, TB), :].astype(F32) * ssmd_ref[:, cs]
                y_ref[pl.ds(t0, TB), cs] = yb.astype(BF16)
                return 0

            def inv_retile(i, c):
                for m in range(3):
                    for cp in w_copies(cc, m, i):
                        cp.wait()
                unrolled(inv_block)(i, c)
                for m in range(3):
                    retile(m, i, cc)

                @pl.when(cc + 1 < n_cc)
                def _():
                    for m in range(3):
                        for cp in w_copies(cc + 1, m, i):
                            cp.start()

                return c

            assert NB // UNR == cpg
            jax.lax.fori_loop(0, cpg, inv_retile, 0)
            return 0

        for cc in range(n_cc):
            chunk(cc, 0)

        wo_retile(n_cc - 2)
        wo_retile(n_cc - 1)
        x_copies[0].wait()

    pl.run_scoped(
        phase_a,
        pltpu.VMEM((KPAD + S, D), BF16), pltpu.VMEM((S, D), BF16), pltpu.VMEM((D, S), BF16),
        pltpu.VMEM((S, CC), BF16),
        pltpu.VMEM((NB, 2 * TB, CC), F32), pltpu.VMEM((NB, 2 * TB, CC), F32),
        pltpu.VMEM((NB, 2 * TB, CC), F32),
        pltpu.VMEM((3 * (CC // DCH), DCH // 2, 2 * NH, DH), BF16), pltpu.VMEM((3, 2, DCH // 2 * WPITCH, DH), U32), pltpu.VMEM((NH * DH, D), BF16),
    )

    scale = DH ** -0.5
    row = jax.lax.broadcasted_iota(jnp.int32, (L, L), 0)
    col = jax.lax.broadcasted_iota(jnp.int32, (L, L), 1)
    mask = (row < MEM) | (row >= col)

    def out_copy(t):
        r = pl.multiple_of(t * (SEG * SUNR), SEG * SUNR)
        return pltpu.make_async_copy(out_ref.at[pl.ds(r, SEG * SUNR), :], o_hbm.at[pl.ds(r, SEG * SUNR), :], sem_out)

    def epilogue(s, b):
        r = pl.multiple_of(s * SEG, SEG)
        xs = x_ref[pl.ds(r, SEG), :].astype(F32)
        gsum = jnp.sum((xs * gate_ref[...]).astype(BF16).astype(F32), axis=-1, keepdims=True)
        gte = jax.nn.sigmoid(gsum.astype(BF16).astype(F32))
        a = (xs * y_ref[pl.ds(r, SEG), :].astype(F32)).astype(BF16).astype(F32)
        out_ref[pl.ds(r, SEG), :] = (gte * a + (1.0 - gte) * b.astype(F32)).astype(BF16)

    def seg_body(s, mem):
        r = pl.multiple_of(s * SEG, SEG)
        xs = x_ref[pl.ds(r, SEG), :].astype(F32)
        h = jnp.concatenate([mem, xs], axis=0)
        qkvs = [None] * NH
        ps = [None] * NH
        os_ = [None] * NH

        def probs(hd):
            q = qkvs[hd][:, 0:DH].astype(BF16).astype(F32)
            k = qkvs[hd][:, DH:2 * DH].astype(BF16)
            sc = jnp.where(mask, _nt(q, k) * scale, -1e9)
            e = jnp.exp(sc - jnp.max(sc, axis=-1, keepdims=True))
            ps[hd] = (e / jnp.sum(e, axis=-1, keepdims=True)).astype(BF16).astype(F32)

        def values(hd):
            o = _nn(ps[hd], qkvs[hd][:, 2 * DH:3 * DH].astype(BF16))
            os_[hd] = o.astype(BF16).astype(F32)

        def slot(g):
            if g < NH:
                qkvs[g] = _nn(h, pltpu.bitcast(w2_ref[:, pl.ds(g * 3 * DH, 3 * DH)], BF16))
            if 0 <= g - L1 < NH:
                probs(g - L1)
            if 0 <= g - L2 < NH:
                values(g - L2)

        for g in range(NH):
            slot(g)
        acc = None
        nxt = NH
        for w in range(NH // WOG):
            while nxt < NH + L2 and (nxt - NH < w + 1 - TOFF or nxt - L2 < (w + 1) * WOG):
                slot(nxt)
                nxt += 1
            og = jnp.concatenate(os_[w * WOG:(w + 1) * WOG], axis=1)
            wog = pltpu.bitcast(wo2_ref[pl.ds(w * WOG * DH // 2, WOG * DH // 2), :], BF16)
            part = _nn(og, wog)
            acc = part if acc is None else acc + part
        ob = acc.astype(BF16)
        epilogue(s, ob[MEM:])
        return ob[:MEM].astype(F32)

    def seg_pair(t, mem):
        @pl.when(t == XSPLIT // (SEG * SUNR))
        def _():
            x_copies[1].wait()

        for u in range(SUNR):
            mem = seg_body(t * SUNR + u, mem)
        out_copy(t).start()
        return mem

    jax.lax.fori_loop(0, NSEG // SUNR, seg_pair, mem0_ref[...].astype(F32))
    pltpu.make_async_copy(out_ref, o_hbm, sem_out).wait()


@functools.partial(jax.jit, static_argnames=("B_seg_len",))
def pallas_gated_mix__ssm_conv_h3__memory_aug_recurrent_mem_tr__prompt_kernel(
    A_q, A_k, A_v, A_shift_k, A_ssm_k, A_ssm_D, B_x, B_mem0, B_Wq, B_Wk, B_Wv, B_Wo, B_seg_len, gate_w,
):
    del B_x
    assert B_seg_len == SEG
    fwd, inv, sgn = _dft_consts()
    any_spec = pl.BlockSpec(memory_space=pl.ANY)
    vmem_spec = pl.BlockSpec(memory_space=pltpu.VMEM)
    out = pl.pallas_call(
        _kernel,
        out_shape=jax.ShapeDtypeStruct((S, D), BF16),
        in_specs=[any_spec] * 8 + [vmem_spec] * 7,
        out_specs=any_spec,
        scratch_shapes=[
            pltpu.VMEM((S, D), BF16),
            pltpu.VMEM((S, D), BF16),
            pltpu.VMEM((D // 2, 3 * NH * DH), U32),
            pltpu.VMEM((NH * DH // 2, D), U32),
            pltpu.VMEM((S, D), BF16),
            pltpu.VMEM((1, D), F32),
            pltpu.VMEM((1, D), F32),
            pltpu.SemaphoreType.DMA((3 * (D // CC),)),
            pltpu.SemaphoreType.DMA((3 * (CC // DCH) + D // CC,)),
            pltpu.SemaphoreType.DMA((2,)),
            pltpu.SemaphoreType.DMA(()),
        ],
        compiler_params=pltpu.CompilerParams(vmem_limit_bytes=120 * 1024 * 1024),
    )(
        A_q.reshape(S, D), A_k.reshape(S, D), A_v.reshape(S, D), A_ssm_k,
        B_Wq.reshape(D // 2, 2 * NH, DH), B_Wk.reshape(D // 2, 2 * NH, DH), B_Wv.reshape(D // 2, 2 * NH, DH),
        B_Wo.reshape(NH * DH, D),
        A_shift_k.T, A_ssm_D, gate_w, B_mem0.reshape(MEM, D),
        jnp.asarray(fwd.astype(jnp.bfloat16)), jnp.asarray(inv.astype(jnp.bfloat16)), jnp.asarray(sgn),
    )
    return out.reshape(1, S, D)
```
